```python
import os as _os
_os.environ.setdefault("JAX_PLATFORMS", "cpu")
import jax
import jax.numpy as jnp

def _softmax(x, axis=-1):
    return jax.nn.softmax(x, axis=axis)
def _gelu(x):
    return jax.nn.gelu(x, approximate=True)
def _silu(x):
    return jax.nn.silu(x)
def _sigmoid(x):
    return jax.nn.sigmoid(x)
def _layernorm(x, axis=-1, eps=1e-5):
    m = jnp.mean(x, axis=axis, keepdims=True)
    v = jnp.var(x, axis=axis, keepdims=True)
    return (x - m) / jnp.sqrt(v + eps)
def _scatter_add(tgt, idx, src, axis=0):
    return tgt.at[idx].add(src)
def _segment_sum(src, seg, n):
    return jax.ops.segment_sum(src, seg, n)
class _Rng:
    def __init__(self, key):
        self._k = key
    def _next(self):
        self._k, sub = jax.random.split(self._k)
        return sub
    def normal(self, shape):
        return jax.random.normal(self._next(), shape, dtype=jnp.bfloat16)
    def randint(self, lo, hi, shape):
        return jax.random.randint(self._next(), shape, lo, hi, dtype=jnp.int32)
    def uniform(self, shape, lo=0.0, hi=1.0):
        return jax.random.uniform(self._next(), shape, jnp.bfloat16, lo, hi)
    def permutation(self, n):
        return jax.random.permutation(self._next(), n)


kernel_name = 'interleave_layers__linear_attn_block__mha_block__prompt'

def setup_inputs():
    _rng = _Rng(jax.random.key(int.from_bytes(__import__("os").urandom(4), "little")))
    _w = (lambda a: (lambda t: t.astype(jnp.bfloat16) if jnp.issubdtype(t.dtype, jnp.floating) else t)(jnp.asarray(a)))
    def _A_setup():
        B, S, D = 1, 2048, 640
        return {
            "x": _w((lambda *s: _rng.normal(s) * 0.05)(B, S, D)),
            "wqkv": _w((lambda *s: _rng.normal(s) * 0.1)(D, 3 * D)),
            "wo": _w((lambda *s: _rng.normal(s) * 0.05)(D, D)),
        }
    _A_in = _A_setup()

    def _B_setup():
        B, S, D, H = 1, 2048, 640, 32
        return {
            "x": _w((lambda *s: _rng.normal(s) * 0.05)(B, S, D)),
            "wqkv": _w((lambda *s: _rng.normal(s) * 0.1)(D, 3 * D)),
            "wo": _w((lambda *s: _rng.normal(s) * 0.05)(D, D)),
        }
    _B_in = _B_setup()

    return {
        "A_x": _A_in["x"],
        "A_wqkv": _A_in["wqkv"],
        "A_wo": _A_in["wo"],
        "B_x": _B_in["x"],
        "B_wqkv": _B_in["wqkv"],
        "B_wo": _B_in["wo"],
    }

def reference(A_x, A_wqkv, A_wo, B_x, B_wqkv, B_wo):
    def _A_ref(x, wqkv, wo):
        B, S, D = x.shape
        H = 32; Dh = D // H
        qkv = (lambda x, *d: x.transpose(*d))((x @ wqkv).reshape(B, S, 3, H, Dh), 2, 0, 3, 1, 4)
        q, k, v = qkv[0], qkv[1], qkv[2]
        phi = lambda t: jnp.where(t > 0, t + 1, jnp.exp(t)) + 1e-6
        pq, pk = phi(q), phi(k)
        kv = jnp.einsum("bhsd,bhse->bhde", pk, v)
        z = jnp.einsum("bhsd->bhd", pk)
        num = jnp.einsum("bhqd,bhde->bhqe", pq, kv)
        den = jnp.einsum("bhqd,bhd->bhq", pq, z)[..., None] + 1e-6
        o = num / den
        return (lambda x, *d: x.transpose(*d))(o, 0, 2, 1, 3).reshape(B, S, D) @ wo

    def _B_ref(x, wqkv, wo):
        B, S, D = x.shape
        H = 32
        Dh = D // H
        qkv = (lambda x, *d: x.transpose(*d))((x @ wqkv).reshape(B, S, 3, H, Dh), 2, 0, 3, 1, 4)
        q, k, v = qkv[0], qkv[1], qkv[2]
        scores = jnp.einsum("bhqd,bhkd->bhqk", q, k) * (Dh ** -0.5)
        p = _softmax(scores, axis=-1)
        o = jnp.einsum("bhqk,bhkd->bhqd", p, v)
        return (lambda x, *d: x.transpose(*d))(o, 0, 2, 1, 3).reshape(B, S, D) @ wo

    x = A_x
    x = x + _A_ref(_layernorm(x, axis=-1), A_wqkv, A_wo)
    x = x + _B_ref(_layernorm(x, axis=-1), B_wqkv, B_wo)
    x = x + _A_ref(_layernorm(x, axis=-1), A_wqkv, A_wo)
    x = x + _B_ref(_layernorm(x, axis=-1), B_wqkv, B_wo)
    return x
```

```python
import jax
import jax.numpy as jnp
from jax import lax
import jax.experimental.pallas as pl
import jax.experimental.pallas.tpu as pltpu

S = 2048
D = 640
H = 32
DH = 20
NTILE = D // 128
RB = 256
NRB = S // RB
TQ = 256
TK = 128
NQ = S // TQ
NC = S // TK
VROWS = 24

LOG2E = 1.4426950408889634
QSCALE = (DH ** -0.5) * LOG2E

F32 = jnp.float32
BF16 = jnp.bfloat16
_NT = (((1,), (1,)), ((), ()))


def _dot(a, b):
    return jnp.dot(a, b, preferred_element_type=F32)


def _dot_nt(a, b):
    return lax.dot_general(a, b, _NT, preferred_element_type=F32)


def _layernorm(xb):
    m = jnp.mean(xb, axis=-1, keepdims=True)
    xc = xb - m
    v = jnp.mean(xc * xc, axis=-1, keepdims=True)
    return xc * lax.rsqrt(v + 1e-5)


def _phi(t):
    return jnp.where(t > 0, t + 1.0, jnp.exp(t)) + 1e-6


def _kernel(x_in, wa_ref, wao_ref, wb_ref, wbo_ref, out_ref,
            x_ref, wakt_ref, wbqvt_ref, pq_ref, g_ref, zp_ref, m_ref, z64_ref, e_ref,
            qt_ref, k_ref, vt_ref, ot_ref, s_ref, mx_ref):
    x_ref[...] = x_in[...].astype(F32)
    wakt_ref[...] = wa_ref[:, D:2 * D].astype(F32).T.astype(BF16)
    wbqvt_ref[0:D, :] = wb_ref[:, 0:D].astype(F32).T.astype(BF16)
    wbqvt_ref[D:2 * D, :] = wb_ref[:, 2 * D:3 * D].astype(F32).T.astype(BF16)
    ej = lax.broadcasted_iota(jnp.int32, (128, D), 0)
    ee = lax.broadcasted_iota(jnp.int32, (128, D), 1)
    ejh = (ej & 31) * DH
    e_ref[...] = jnp.where((ej < 64) & (ee >= ejh) & (ee < ejh + DH), 1.0, 0.0).astype(BF16)

    def rows_of(i):
        return pl.ds(pl.multiple_of(i * RB, RB), RB)

    def layer_a():
        g_ref[...] = jnp.zeros(g_ref.shape, F32)
        zp_ref[...] = jnp.zeros(zp_ref.shape, F32)

        def a1(i, c):
            rows = rows_of(i)
            xn = _layernorm(x_ref[rows, :]).astype(BF16)
            pq_ref[rows, :] = _phi(_dot(xn, wa_ref[:, 0:D])).astype(BF16)
            pkt = _phi(_dot_nt(wakt_ref[...], xn))
            zp = pkt[:, 0:128]
            for t in range(1, RB // 128):
                zp = zp + pkt[:, t * 128:(t + 1) * 128]
            zp_ref[...] += zp
            g_ref[...] += _dot(pkt.astype(BF16), xn)
            return c
        lax.fori_loop(0, NRB, a1, 0)

        kv = _dot(g_ref[...].astype(BF16), wa_ref[:, 2 * D:3 * D])
        rd = lax.broadcasted_iota(jnp.int32, (D, D), 0)
        ce = lax.broadcasted_iota(jnp.int32, (D, D), 1)
        rh = (rd * 3277) >> 16
        lo = rh * DH
        kvm = jnp.where((ce >= lo) & (ce < lo + DH), kv, 0.0).astype(BF16)
        m_ref[...] = _dot(kvm, wao_ref[...]).astype(BF16)
        z = jnp.sum(zp_ref[...], axis=1, keepdims=True)
        rd2 = lax.broadcasted_iota(jnp.int32, (D, 128), 0)
        cj = lax.broadcasted_iota(jnp.int32, (D, 128), 1)
        rh2 = (rd2 * 3277) >> 16
        z64_ref[...] = jnp.where((cj < 64) & ((cj & 31) == rh2), z, 0.0).astype(BF16)

        def a3(i, c):
            rows = rows_of(i)
            pq = pq_ref[rows, :]
            den = _dot(pq, z64_ref[...]) + 1e-6
            r = 1.0 / den
            r_hi = r.astype(BF16).astype(F32)
            lane = lax.broadcasted_iota(jnp.int32, (RB, 128), 1)
            r2 = jnp.where(lane < 32, r_hi, jnp.where(lane < 64, r - r_hi, 0.0)).astype(BF16)
            r_exp = _dot(r2, e_ref[...])
            y = (pq.astype(F32) * r_exp).astype(BF16)
            x_ref[rows, :] += _dot(y, m_ref[...])
            return c
        lax.fori_loop(0, NRB, a3, 0)

    def layer_b():
        def b1(i, c):
            rows = rows_of(i)
            xn = _layernorm(x_ref[rows, :]).astype(BF16)
            k = _dot(xn, wb_ref[:, D:2 * D])
            lane = lax.broadcasted_iota(jnp.int32, (RB, 128), 1)
            for t in range(NTILE):
                k_ref[t, rows, :] = k[:, t * 128:(t + 1) * 128].astype(BF16)
            for t in range(NTILE - 1):
                k_ref[NTILE + t, rows, :] = jnp.where(
                    lane >= 64, k[:, t * 128:(t + 1) * 128],
                    k[:, (t + 1) * 128:(t + 2) * 128]).astype(BF16)
            qvt = _dot_nt(wbqvt_ref[...], xn)
            qt_ref[:, rows] = qvt[0:D, :] * QSCALE
            vt_ref[:, rows] = qvt[D:2 * D, :]
            return c
        lax.fori_loop(0, NRB, b1, 0)

        def attn(h1, h2):
            if h1 is not None:
                d0 = h1 * DH
                t = d0 >> 7
                lo = d0 & 127
                ktile = jnp.where(lo > 128 - DH, NTILE + t, t)
                t_hi = pl.multiple_of(t * 128, 128)
                t_lo = pl.multiple_of(jnp.minimum(t + 1, NTILE - 1) * 128, 128)
                r = lax.broadcasted_iota(jnp.int32, (128, TQ), 0)
                in_head = ((r - lo) & 127) < DH
                upper = r >= lo
            if h2 is not None:
                d2 = h2 * DH
                w0 = pl.multiple_of((d2 >> 3) << 3, 8)
                off = d2 - w0
                rv = lax.broadcasted_iota(jnp.int32, (VROWS, S), 0)
                vt = jnp.where((rv >= off) & (rv < off + DH), vt_ref[pl.ds(w0, VROWS), :], 1.0)
                ro = lax.broadcasted_iota(jnp.int32, (VROWS, TQ), 0)
                ovalid = (ro >= off) & (ro < off + DH)
            for u in range(NQ):
                cols = slice(u * TQ, (u + 1) * TQ)
                if h1 is not None:
                    qw = jnp.where(upper, qt_ref[pl.ds(t_hi, 128), cols], qt_ref[pl.ds(t_lo, 128), cols])
                    qw = jnp.where(in_head, qw, 0.0).astype(BF16)
                if h2 is not None:
                    m2 = mx_ref[u]
                m = None
                acc = None
                for c in range(NC):
                    ks = slice(c * TK, (c + 1) * TK)
                    if h2 is not None:
                        s = s_ref[u, ks, :]
                        p = jnp.exp2(s.reshape(TK // 8, 8, TQ) - m2[None]).reshape(TK, TQ)
                        d = _dot(vt[:, ks], p)
                        acc = d if acc is None else acc + d
                    if h1 is not None:
                        s = _dot(k_ref[ktile, ks, :], qw)
                        s_ref[u, ks, :] = s
                        mc = jnp.max(s.reshape(TK // 8, 8, TQ), axis=0)
                        m = mc if m is None else jnp.maximum(m, mc)
                if h1 is not None:
                    m = jnp.max(m, axis=0, keepdims=True)
                    mx_ref[u] = jnp.broadcast_to(m, (8, TQ))
                if h2 is not None:
                    l = jnp.where(off == 0, acc[DH:DH + 1, :], acc[0:1, :])
                    o = acc / l
                    pltpu.store(ot_ref.at[pl.ds(w0, VROWS), cols], o, mask=ovalid)

        attn(0, None)

        def body(h, c):
            attn(h + 1, h)
            return c
        lax.fori_loop(0, H - 1, body, 0)
        attn(None, H - 1)

        def b3(i, c):
            rows = rows_of(i)
            o = ot_ref[:, rows].T.astype(BF16)
            x_ref[rows, :] += _dot(o, wbo_ref[...])
            return c
        lax.fori_loop(0, NRB, b3, 0)

    def two_layers(it, c):
        layer_a()
        layer_b()
        return c
    lax.fori_loop(0, 2, two_layers, 0)
    out_ref[...] = x_ref[...].astype(BF16)


@jax.jit
def pallas_interleave_layers__linear_attn_block__mha_block__prompt_kernel(
    A_x: jax.Array,
    A_wqkv: jax.Array,
    A_wo: jax.Array,
    B_x: jax.Array,
    B_wqkv: jax.Array,
    B_wo: jax.Array,
):
    del B_x
    x = A_x.reshape(S, D)
    out = pl.pallas_call(
        _kernel,
        out_shape=jax.ShapeDtypeStruct((S, D), BF16),
        scratch_shapes=[
            pltpu.VMEM((S, D), F32),
            pltpu.VMEM((D, D), BF16),
            pltpu.VMEM((2 * D, D), BF16),
            pltpu.VMEM((S, D), BF16),
            pltpu.VMEM((D, D), F32),
            pltpu.VMEM((D, 128), F32),
            pltpu.VMEM((D, D), BF16),
            pltpu.VMEM((D, 128), BF16),
            pltpu.VMEM((128, D), BF16),
            pltpu.VMEM((D, S), F32),
            pltpu.VMEM((2 * NTILE - 1, S, 128), BF16),
            pltpu.VMEM((D, S), F32),
            pltpu.VMEM((D, S), F32),
            pltpu.VMEM((NQ, S, TQ), F32),
            pltpu.VMEM((NQ, 8, TQ), F32),
        ],
        compiler_params=pltpu.CompilerParams(vmem_limit_bytes=110 * 1024 * 1024),
    )(x, A_wqkv, A_wo, B_wqkv, B_wo)
    return out.reshape(1, S, D)
```

```python
import jax
import jax.numpy as jnp
from jax import lax
import jax.experimental.pallas as pl
import jax.experimental.pallas.tpu as pltpu

S = 2048
D = 640
H = 32
DH = 20
NTILE = D // 128
RB = 256
NB = S // RB
NIT = NB // 2
TQ = 256
TK = 128
NQ = S // TQ
NC = S // TK
VROWS = 24
KV_ROWS = ((0, 144), (112, 272), (240, 400), (368, 528), (496, 640))

LOG2E = 1.4426950408889634
QSCALE = (DH ** -0.5) * LOG2E

F32 = jnp.float32
BF16 = jnp.bfloat16
_NT = (((1,), (1,)), ((), ()))


def _dot(a, b):
    return jnp.dot(a, b, preferred_element_type=F32)


def _dot_nt(a, b):
    return lax.dot_general(a, b, _NT, preferred_element_type=F32)


def _layernorm(xb):
    m = jnp.mean(xb, axis=-1, keepdims=True)
    xc = xb - m
    v = jnp.mean(xc * xc, axis=-1, keepdims=True)
    return (xc * lax.rsqrt(v + 1e-5)).astype(BF16)


def _phi(t):
    return jnp.where(t > 0, t + 1.0, jnp.exp(t)) + 1e-6


def _kernel(x_hbm, wa_hbm, wao_hbm, wb_hbm, wbo_hbm, out_hbm,
            xin_ref, wa_ref, wao_ref, wb_ref, wbo_ref, sems,
            x_ref, xn_ref, wat_ref, wbt_ref, pq_ref, g_ref, zp_ref, m_ref, zh_ref,
            qt_ref, k_ref, vt_ref, ot_ref, s_ref, mx_ref):

    def rows_of(b):
        if isinstance(b, int):
            return slice(b * RB, (b + 1) * RB)
        return pl.ds(pl.multiple_of(b * RB, RB), RB)

    def x_copy(b):
        return pltpu.make_async_copy(x_hbm.at[rows_of(b), :], xin_ref.at[rows_of(b), :], sems.at[b])

    def out_copy(b):
        return pltpu.make_async_copy(xin_ref.at[rows_of(b), :], out_hbm.at[rows_of(b), :], sems.at[b])

    cp_wak = pltpu.make_async_copy(wa_hbm.at[:, pl.ds(D, D)], wa_ref.at[:, pl.ds(D, D)], sems.at[NB])
    cp_waq = pltpu.make_async_copy(wa_hbm.at[:, pl.ds(0, D)], wa_ref.at[:, pl.ds(0, D)], sems.at[NB + 1])
    cp_wav = pltpu.make_async_copy(wa_hbm.at[:, pl.ds(2 * D, D)], wa_ref.at[:, pl.ds(2 * D, D)],
                                   sems.at[NB + 2])
    cp_wao = pltpu.make_async_copy(wao_hbm, wao_ref, sems.at[NB + 3])
    cp_wb = pltpu.make_async_copy(wb_hbm, wb_ref, sems.at[NB + 4])
    cp_wbo = pltpu.make_async_copy(wbo_hbm, wbo_ref, sems.at[NB + 5])

    def a1_stage(b, xn):
        pkt = _phi(_dot_nt(wat_ref[0:D, :], xn))
        pq_ref[:, rows_of(b)] = _phi(_dot_nt(wat_ref[D:2 * D, :], xn))
        zp = pkt[:, 0:128]
        for t in range(1, RB // 128):
            zp = zp + pkt[:, t * 128:(t + 1) * 128]
        return zp, _dot(pkt.astype(BF16), xn)

    def a1_pair(j, ln_of):
        xn_b = ln_of(2 * j + 1)
        zp0, g0 = a1_stage(2 * j, xn_ref[...])
        xn_ref[...] = ln_of(jnp.minimum(2 * j + 2, NB - 1))
        zp1, g1 = a1_stage(2 * j + 1, xn_b)
        zp_ref[...] += zp0 + zp1
        g_ref[...] += g0 + g1

    def a2():
        z = jnp.sum(zp_ref[...].T, axis=0, keepdims=True)
        hj = lax.broadcasted_iota(jnp.int32, (H, D), 0) * DH
        cd = lax.broadcasted_iota(jnp.int32, (H, D), 1)
        zh_ref[...] = jnp.where((cd >= hj) & (cd < hj + DH), z, 0.0)
        kvm = []
        for t, (lo, hi) in enumerate(KV_ROWS):
            n = hi - lo
            kv = _dot(g_ref[lo:hi, :].astype(BF16), wa_ref[:, 2 * D + t * 128:2 * D + (t + 1) * 128])
            rd = lax.broadcasted_iota(jnp.int32, (n, 128), 0) + lo
            ce = lax.broadcasted_iota(jnp.int32, (n, 128), 1) + t * 128
            h0 = ((rd * 3277) >> 16) * DH
            kvm.append(jnp.where((ce >= h0) & (ce < h0 + DH), kv, 0.0).astype(BF16))
        y0 = a3_y(0)
        mt = [_dot(kvm[t], wao_ref[t * 128:(t + 1) * 128, :]) for t in range(NTILE)]
        for t, (lo, hi) in enumerate(KV_ROWS):
            a = KV_ROWS[t - 1][1] if t > 0 else lo
            b = KV_ROWS[t + 1][0] if t + 1 < NTILE else hi
            m_ref[a:b, :] = mt[t][a - lo:b - lo, :].astype(BF16)
            if b < hi:
                m_ref[b:hi, :] = (mt[t][b - lo:, :] + mt[t + 1][0:hi - b, :]).astype(BF16)
        g_ref[...] = jnp.zeros(g_ref.shape, F32)
        zp_ref[...] = jnp.zeros(zp_ref.shape, F32)
        return y0

    def a3_y(b):
        rows = rows_of(b)
        r = 1.0 / (_dot(zh_ref[...], pq_ref[:, rows]) + 1e-6)
        sub = lax.broadcasted_iota(jnp.int32, (8, RB), 0)
        pieces = []
        for j in range(H // 2):
            ra = jnp.broadcast_to(r[2 * j:2 * j + 1, :], (8, RB))
            rb = jnp.broadcast_to(r[2 * j + 1:2 * j + 2, :], (8, RB))
            pieces += [ra, ra, jnp.where(sub < 4, ra, rb), rb, rb]
        return (pq_ref[:, rows] * jnp.concatenate(pieces, axis=0)).T.astype(BF16)

    def a3_x(b, y):
        xb = x_ref[rows_of(b), :] + _dot(y, m_ref[...])
        x_ref[rows_of(b), :] = xb
        return xb

    def b1_k(b, xn):
        rows = rows_of(b)
        k = _dot(xn, wb_ref[:, D:2 * D])
        lane = lax.broadcasted_iota(jnp.int32, (RB, 128), 1)
        for t in range(NTILE):
            k_ref[t, rows, :] = k[:, t * 128:(t + 1) * 128].astype(BF16)
        for t in range(NTILE - 1):
            k_ref[NTILE + t, rows, :] = jnp.where(
                lane >= 64, k[:, t * 128:(t + 1) * 128],
                k[:, (t + 1) * 128:(t + 2) * 128]).astype(BF16)

    def b1_qv(b, xn):
        rows = rows_of(b)
        qvt = _dot_nt(wbt_ref[...], xn)
        qt_ref[:, rows] = qvt[0:D, :] * QSCALE
        vt_ref[:, rows] = qvt[D:2 * D, :]

    def attn(h1, h2, par, extra=None, blocks=None):
        if h1 is not None:
            d0 = h1 * DH
            t = d0 >> 7
            lo = d0 & 127
            ktile = jnp.where(lo > 128 - DH, NTILE + t, t)
            t_hi = pl.multiple_of(t * 128, 128)
            t_lo = pl.multiple_of(jnp.minimum(t + 1, NTILE - 1) * 128, 128)
            r = lax.broadcasted_iota(jnp.int32, (128, TQ), 0)
            in_head = ((r - lo) & 127) < DH
            upper = r >= lo
        if h2 is not None:
            off = 4 * par
            w0 = pl.multiple_of(h2 * DH - off, 8)
            rv = lax.broadcasted_iota(jnp.int32, (VROWS, S), 0)
            vt = jnp.where((rv >= off) & (rv < off + DH), vt_ref[pl.ds(w0, VROWS), :], 1.0)
            ro = lax.broadcasted_iota(jnp.int32, (VROWS, TQ), 0)
            ovalid = (ro >= off) & (ro < off + DH)
            lrow = DH if par == 0 else 0
        for u in (range(NQ) if blocks is None else blocks):
            cols = rows_of(u)
            if h1 is not None:
                qw = jnp.where(upper, qt_ref[pl.ds(t_hi, 128), cols], qt_ref[pl.ds(t_lo, 128), cols])
                qw = jnp.where(in_head, qw, 0.0).astype(BF16)
            if h2 is not None:
                m2 = mx_ref[par, u]
            m = None
            acc = None
            for c in range(NC):
                ks = slice(c * TK, (c + 1) * TK)
                if h2 is not None:
                    s = s_ref[par, u, ks, :]
                    p = jnp.exp2(s.reshape(TK // 8, 8, TQ) - m2[None]).reshape(TK, TQ)
                    d = _dot(vt[:, ks], p)
                    acc = d if acc is None else acc + d
                if h1 is not None:
                    s = _dot(k_ref[ktile, ks, :], qw)
                    s_ref[par, u, ks, :] = s
                    mc = jnp.max(s.reshape(TK // 8, 8, TQ), axis=0)
                    m = mc if m is None else jnp.maximum(m, mc)
                if extra is not None:
                    extra(u, c)
            if h1 is not None:
                m = jnp.max(m, axis=0, keepdims=True)
                mx_ref[par, u] = jnp.broadcast_to(m, (8, TQ))
            if h2 is not None:
                o = acc / acc[lrow:lrow + 1, :]
                pltpu.store(ot_ref.at[pl.ds(w0, VROWS), cols], o, mask=ovalid)

    def last_heads(u):
        base = pl.multiple_of(u * RB, RB)
        half = [pl.ds(base + i * 128, 128) for i in range(2)]
        o = [ot_ref[0:512, r].T.astype(BF16) for r in half]
        pieces = [(i, n, k) for k in range(2) for i in range(2) for n in range(NTILE)]

        def piece(j):
            i, n, k = pieces[j]
            x_ref[half[i], n * 128:(n + 1) * 128] += _dot(
                o[i][:, k * 256:(k + 1) * 256], wbo_ref[k * 256:(k + 1) * 256, n * 128:(n + 1) * 128])
        slots = (0, 2, 4, 7, 9, 11, 14, 16, 18, 21, 23, 25, 28, 30)

        def extra(first):
            def f(_, c):
                if first + c in slots:
                    piece(slots.index(first + c))
            return f
        attn(None, H - 2, 0, extra(0), blocks=[u])
        attn(None, H - 1, 1, extra(NC), blocks=[u])
        for j in range(len(slots), len(pieces)):
            piece(j)
        rows = rows_of(u)
        xb = x_ref[rows, :] + _dot(ot_ref[512:D, rows].T.astype(BF16), wbo_ref[512:D, :])
        x_ref[rows, :] = xb
        xin_ref[rows, :] = xb.astype(BF16)
        out_copy(u).start()

    cp_wak.start()
    x_copy(0).start()
    cp_waq.start()
    x_copy(1).start()
    x_copy(2).start()
    g_ref[...] = jnp.zeros(g_ref.shape, F32)
    zp_ref[...] = jnp.zeros(zp_ref.shape, F32)
    cp_wak.wait()
    for b in range(3, NB):
        x_copy(b).start()
    cp_wav.start()
    cp_wao.start()
    cp_wb.start()
    cp_wbo.start()
    wat_ref[0:D, :] = wa_ref[:, D:2 * D].astype(F32).T.astype(BF16)
    x_copy(0).wait()
    x0 = xin_ref[rows_of(0), :].astype(F32)
    x_ref[rows_of(0), :] = x0
    xn_ref[...] = _layernorm(x0)
    cp_waq.wait()
    wat_ref[D:2 * D, :] = wa_ref[:, 0:D].astype(F32).T.astype(BF16)

    def two_layers(it, c):
        first = it == 0

        def load_x(b):
            rows = rows_of(b)
            xb = jnp.where(first, xin_ref[rows, :].astype(F32), x_ref[rows, :])
            x_ref[rows, :] = xb
            return _layernorm(xb)

        def a1_body(j, c):
            @pl.when(first)
            def _():
                x_copy(2 * j + 1).wait()

                @pl.when(j < NIT - 1)
                def _():
                    x_copy(2 * j + 2).wait()
            a1_pair(j, load_x)
            return c
        lax.fori_loop(0, NIT, a1_body, 0)

        @pl.when(first)
        def _():
            cp_wav.wait()
            cp_wao.wait()
            cp_wb.wait()
            cp_wbo.wait()

        @pl.when(jnp.logical_not(first))
        def _():
            for b in range(NB):
                out_copy(b).wait()

        wbt_ref[0:D, :] = wb_ref[:, 0:D].astype(F32).T.astype(BF16)
        wbt_ref[D:2 * D, :] = wb_ref[:, 2 * D:3 * D].astype(F32).T.astype(BF16)
        xn_ref[...] = _layernorm(a3_x(0, a2()))

        def a3_b1(b, c):
            y = a3_y(b + 1)
            b1_k(b, xn_ref[...])
            xn_next = _layernorm(a3_x(b + 1, y))
            b1_qv(b, xn_ref[...])
            xn_ref[...] = xn_next
            return c
        lax.fori_loop(0, NB - 1, a3_b1, 0)
        b1_k(NB - 1, xn_ref[...])
        b1_qv(NB - 1, xn_ref[...])

        def first_scores(h, c):
            attn(h, None, h)
            return c
        lax.fori_loop(0, 2, first_scores, 0)

        def body(i, c):
            attn(2 * i + 2, 2 * i, 0)
            attn(2 * i + 3, 2 * i + 1, 1)
            return c
        lax.fori_loop(0, H // 2 - 1, body, 0)

        def tail(j, c):
            last_heads(2 * j)
            last_heads(2 * j + 1)
            return c
        lax.fori_loop(0, NIT, tail, 0)

        @pl.when(first)
        def _():
            xn_ref[...] = _layernorm(x_ref[rows_of(0), :])
        return c
    lax.fori_loop(0, 2, two_layers, 0)
    for b in range(NB):
        out_copy(b).wait()


@jax.jit
def pallas_interleave_layers__linear_attn_block__mha_block__prompt_kernel(
    A_x: jax.Array,
    A_wqkv: jax.Array,
    A_wo: jax.Array,
    B_x: jax.Array,
    B_wqkv: jax.Array,
    B_wo: jax.Array,
):
    del B_x
    x = A_x.reshape(S, D)
    any_spec = pl.BlockSpec(memory_space=pl.ANY)
    out = pl.pallas_call(
        _kernel,
        out_shape=jax.ShapeDtypeStruct((S, D), BF16),
        in_specs=[any_spec] * 5,
        out_specs=any_spec,
        scratch_shapes=[
            pltpu.VMEM((S, D), BF16),
            pltpu.VMEM((D, 3 * D), BF16),
            pltpu.VMEM((D, D), BF16),
            pltpu.VMEM((D, 3 * D), BF16),
            pltpu.VMEM((D, D), BF16),
            pltpu.SemaphoreType.DMA((NB + 6,)),
            pltpu.VMEM((S, D), F32),
            pltpu.VMEM((RB, D), BF16),
            pltpu.VMEM((2 * D, D), BF16),
            pltpu.VMEM((2 * D, D), BF16),
            pltpu.VMEM((D, S), F32),
            pltpu.VMEM((D, D), F32),
            pltpu.VMEM((D, 128), F32),
            pltpu.VMEM((D, D), BF16),
            pltpu.VMEM((H, D), F32),
            pltpu.VMEM((D, S), F32),
            pltpu.VMEM((2 * NTILE - 1, S, 128), BF16),
            pltpu.VMEM((D, S), F32),
            pltpu.VMEM((D, S), F32),
            pltpu.VMEM((2, NQ, S, TQ), F32),
            pltpu.VMEM((2, NQ, 8, TQ), F32),
        ],
        compiler_params=pltpu.CompilerParams(vmem_limit_bytes=110 * 1024 * 1024),
    )(x, A_wqkv, A_wo, B_wqkv, B_wo)
    return out.reshape(1, S, D)
```

```python
import jax
import jax.numpy as jnp
from jax import lax
import jax.experimental.pallas as pl
import jax.experimental.pallas.tpu as pltpu

S = 2048
D = 640
H = 32
DH = 20
NTILE = D // 128
RB = 256
NB = S // RB
NIT = NB // 2
TQ = 128
TK = 128
NQ = S // TQ
NC = S // TK
PACE = 3
VGPAT = (1,)
VG = tuple(VGPAT[c % len(VGPAT)] for c in range(NC))
VGI = tuple(sum(VG[:c]) for c in range(NC))
NVG = sum(VG)
VROWS = 24
KV_ROWS = ((0, 144), (112, 272), (240, 400), (368, 528), (496, 640))

LOG2E = 1.4426950408889634
QSCALE = (DH ** -0.5) * LOG2E

F32 = jnp.float32
BF16 = jnp.bfloat16
_NT = (((1,), (1,)), ((), ()))


def _dot(a, b):
    return jnp.dot(a, b, preferred_element_type=F32)


def _dot_nt(a, b):
    return lax.dot_general(a, b, _NT, preferred_element_type=F32)


def _layernorm(xb):
    m = jnp.mean(xb, axis=-1, keepdims=True)
    xc = xb - m
    v = jnp.mean(xc * xc, axis=-1, keepdims=True)
    return (xc * lax.rsqrt(v + 1e-5)).astype(BF16)


def _phi(t):
    return jnp.where(t > 0, t + 1.0, jnp.exp(t)) + 1e-6


def _kernel(x_hbm, wa_hbm, wao_hbm, wb_hbm, wbo_hbm, out_hbm,
            xin_ref, wa_ref, wao_ref, wb_ref, wbo_ref, sems,
            x_ref, xn_ref, wat_ref, wbt_ref, pq_ref, g_ref, zp_ref, m_ref, zh_ref,
            qt_ref, k_ref, vt_ref, ot_ref, s_ref, mx_ref, qb0_ref, qb1_ref, kb0_ref, kb1_ref, zv_ref, zero_ref):
    qb_refs = (qb0_ref, qb1_ref)
    kb_refs = (kb0_ref, kb1_ref)

    def rows_of(b):
        if isinstance(b, int):
            return slice(b * RB, (b + 1) * RB)
        return pl.ds(pl.multiple_of(b * RB, RB), RB)

    def x_copy(b):
        return pltpu.make_async_copy(x_hbm.at[rows_of(b), :], xin_ref.at[rows_of(b), :], sems.at[b])

    def out_copy(b):
        return pltpu.make_async_copy(xin_ref.at[rows_of(b), :], out_hbm.at[rows_of(b), :], sems.at[b])

    cp_wak = pltpu.make_async_copy(wa_hbm.at[:, pl.ds(D, D)], wa_ref.at[:, pl.ds(D, D)], sems.at[NB])
    cp_waq = pltpu.make_async_copy(wa_hbm.at[:, pl.ds(0, D)], wa_ref.at[:, pl.ds(0, D)], sems.at[NB + 1])
    cp_wav = pltpu.make_async_copy(wa_hbm.at[:, pl.ds(2 * D, D)], wa_ref.at[:, pl.ds(2 * D, D)],
                                   sems.at[NB + 2])
    cp_wao = pltpu.make_async_copy(wao_hbm, wao_ref, sems.at[NB + 3])
    cp_wb = pltpu.make_async_copy(wb_hbm, wb_ref, sems.at[NB + 4])
    cp_wbo = pltpu.make_async_copy(wbo_hbm, wbo_ref, sems.at[NB + 5])

    def a1_stage(b, xn):
        pkt = _phi(_dot_nt(wat_ref[0:D, :], xn))
        pq_ref[:, rows_of(b)] = _phi(_dot_nt(wat_ref[D:2 * D, :], xn))
        zp = pkt[:, 0:128]
        for t in range(1, RB // 128):
            zp = zp + pkt[:, t * 128:(t + 1) * 128]
        return zp, _dot(pkt.astype(BF16), xn)

    def a1_pair(j, ln_of):
        xn_b = ln_of(2 * j + 1)
        zp0, g0 = a1_stage(2 * j, xn_ref[...])
        xn_ref[...] = ln_of(jnp.minimum(2 * j + 2, NB - 1))
        zp1, g1 = a1_stage(2 * j + 1, xn_b)
        zp_ref[...] += zp0 + zp1
        g_ref[...] += g0 + g1

    def a2():
        z = jnp.sum(zp_ref[...].T, axis=0, keepdims=True)
        hj = lax.broadcasted_iota(jnp.int32, (H, D), 0) * DH
        cd = lax.broadcasted_iota(jnp.int32, (H, D), 1)
        zh_ref[...] = jnp.where((cd >= hj) & (cd < hj + DH), z, 0.0)
        kvm = []
        for t, (lo, hi) in enumerate(KV_ROWS):
            n = hi - lo
            kv = _dot(g_ref[lo:hi, :].astype(BF16), wa_ref[:, 2 * D + t * 128:2 * D + (t + 1) * 128])
            rd = lax.broadcasted_iota(jnp.int32, (n, 128), 0) + lo
            ce = lax.broadcasted_iota(jnp.int32, (n, 128), 1) + t * 128
            h0 = ((rd * 3277) >> 16) * DH
            kvm.append(jnp.where((ce >= h0) & (ce < h0 + DH), kv, 0.0).astype(BF16))
        y0 = a3_y(0)
        mt = [_dot(kvm[t], wao_ref[t * 128:(t + 1) * 128, :]) for t in range(NTILE)]
        for t, (lo, hi) in enumerate(KV_ROWS):
            a = KV_ROWS[t - 1][1] if t > 0 else lo
            b = KV_ROWS[t + 1][0] if t + 1 < NTILE else hi
            m_ref[a:b, :] = mt[t][a - lo:b - lo, :].astype(BF16)
            if b < hi:
                m_ref[b:hi, :] = (mt[t][b - lo:, :] + mt[t + 1][0:hi - b, :]).astype(BF16)
        g_ref[...] = jnp.zeros(g_ref.shape, F32)
        zp_ref[...] = jnp.zeros(zp_ref.shape, F32)
        return y0

    def a3_y(b):
        rows = rows_of(b)
        r = 1.0 / (_dot(zh_ref[...], pq_ref[:, rows]) + 1e-6)
        sub = lax.broadcasted_iota(jnp.int32, (8, RB), 0)
        pieces = []
        for j in range(H // 2):
            ra = jnp.broadcast_to(r[2 * j:2 * j + 1, :], (8, RB))
            rb = jnp.broadcast_to(r[2 * j + 1:2 * j + 2, :], (8, RB))
            pieces += [ra, ra, jnp.where(sub < 4, ra, rb), rb, rb]
        return (pq_ref[:, rows] * jnp.concatenate(pieces, axis=0)).T.astype(BF16)

    def a3_x(b, y):
        xb = x_ref[rows_of(b), :] + _dot(y, m_ref[...])
        x_ref[rows_of(b), :] = xb
        return xb

    def b1_k(b, xn):
        rows = rows_of(b)
        k = _dot(xn, wb_ref[:, D:2 * D])
        lane = lax.broadcasted_iota(jnp.int32, (RB, 128), 1)
        for t in range(NTILE):
            k_ref[t, rows, :] = k[:, t * 128:(t + 1) * 128]
        for t in range(NTILE - 1):
            k_ref[NTILE + t, rows, :] = jnp.where(
                lane >= 64, k[:, t * 128:(t + 1) * 128],
                k[:, (t + 1) * 128:(t + 2) * 128])

    def b1_qv(b, xn):
        rows = rows_of(b)
        qvt = _dot_nt(wbt_ref[...], xn)
        for i in range(RB // TQ):
            qs = qvt[0:D, i * TQ:(i + 1) * TQ] * QSCALE
            qt_ref[b * (RB // TQ) + i] = qs
            for par in range(2):
                for dd in range(DH):
                    r = (2 + par) * DH + dd
                    qb_refs[par][b * (RB // TQ) + i, dd] = jnp.broadcast_to(qs[r:r + 1, :], (8, TQ))
        vt_ref[:, rows] = qvt[D:2 * D, :]

    def cols_of(u):
        if isinstance(u, int):
            return slice(u * TQ, (u + 1) * TQ)
        return pl.ds(pl.multiple_of(u * TQ, TQ), TQ)

    def build_qb(h, par, u):
        win = qt_ref[u, pl.ds(pl.multiple_of(h * DH - 4 * par, 8), VROWS), :]
        for dd in range(DH):
            r = 4 * par + dd
            qb_refs[par][u, dd] = jnp.broadcast_to(win[r:r + 1, :], (8, TQ))

    def vpu_keys(h):
        d0 = h * DH
        lo = d0 & 127
        ktile = jnp.where(lo > 128 - DH, NTILE + (d0 >> 7), d0 >> 7)
        rows = jnp.concatenate([k_ref[ktile, c * TK:c * TK + 8 * VG[c], :] for c in range(NC) if VG[c]], axis=0)
        return pltpu.roll(rows, (128 - lo) & 127, axis=1)

    def build_kb(kr, par, ds):
        for dd in ds:
            kbd = jnp.broadcast_to(kr[:, dd:dd + 1], (8 * NVG, TQ))
            for g in range(NVG):
                kb_refs[par][g, dd + zero_ref[0, 0]] = kbd[g * 8:(g + 1) * 8, :]

    def attn(h1, h2, par, extra=None, blocks=None, vpu=False, pace=None):
        if h1 is not None:
            d0 = h1 * DH
            t = d0 >> 7
            lo = d0 & 127
            ktile = jnp.where(lo > 128 - DH, NTILE + t, t)
            t_hi = pl.multiple_of(t * 128, 128)
            t_lo = pl.multiple_of(jnp.minimum(t + 1, NTILE - 1) * 128, 128)
            r = lax.broadcasted_iota(jnp.int32, (128, TQ), 0)
            head_bits = jnp.where(((r - lo) & 127) < DH, -1, zero_ref[0, 0])
            upper = r >= lo
            if vpu:
                kr = vpu_keys(jnp.minimum(h1 + 1, H - 1))
        if h2 is not None:
            off = 4 * par
            w0 = pl.multiple_of(h2 * DH - off, 8)
            rv = lax.broadcasted_iota(jnp.int32, (VROWS, S), 0)
            vt = jnp.where((rv >= off) & (rv < off + DH), vt_ref[pl.ds(w0, VROWS), :], 1.0)
            ro = lax.broadcasted_iota(jnp.int32, (VROWS, TQ), 0)
            ovalid = (ro >= off) & (ro < off + DH)
            lrow = DH if par == 0 else 0
        for ui, u in enumerate(range(NQ) if blocks is None else blocks):
            cols = cols_of(u)
            if h1 is not None:
                qw = jnp.where(upper, qt_ref[u, pl.ds(t_hi, 128), :], qt_ref[u, pl.ds(t_lo, 128), :])
                qw = pltpu.bitcast(pltpu.bitcast(qw, jnp.int32) & head_bits, F32)
            if h2 is not None:
                m2 = mx_ref[par, u]
            m = None
            acc = None
            for c in range(NC):
                ks = slice(c * TK, (c + 1) * TK)
                sv = []
                for g in range(VG[c] if vpu else 0):
                    a = None
                    for dd in range(DH):
                        kb = kb_refs[par][VGI[c] + g, dd]
                        if dd == 0 and len(pace) >= PACE:
                            zs = pltpu.bitcast(pace[-PACE][g * 64:g * 64 + 8, :], jnp.int32) & zv_ref[...]
                            kb = pltpu.bitcast(pltpu.bitcast(kb, jnp.int32) | zs, F32)
                        tt = kb * qb_refs[par][u, dd]
                        a = tt if a is None else a + tt
                    sv.append(a)
                if h2 is not None:
                    s = s_ref[par, u, ks, :]
                    p = jnp.exp2(s.reshape(TK // 8, 8, TQ) - m2[None]).reshape(TK, TQ)
                    d = _dot(vt[:, ks], p)
                    acc = d if acc is None else acc + d
                if h1 is not None:
                    s = _dot(k_ref[ktile, c * TK + 8 * len(sv):(c + 1) * TK, :], qw)
                    if vpu:
                        pace.append(s)
                        s = jnp.concatenate(sv + [s], axis=0)
                    s_ref[par, u, ks, :] = s
                    mc = jnp.max(s.reshape(TK // 8, 8, TQ), axis=0)
                    m = mc if m is None else jnp.maximum(m, mc)
                if extra is not None:
                    extra(ui, c)
            if h1 is not None:
                m = jnp.max(m, axis=0, keepdims=True)
                mx_ref[par, u] = jnp.broadcast_to(m, (8, TQ))
                if vpu:
                    build_qb(jnp.minimum(h1 + 2, H - 2 + par), par, u)
                    if 2 * u < DH:
                        zm = pltpu.bitcast(jnp.broadcast_to(m, (8, TQ)), jnp.int32) & zv_ref[...]
                        krz = pltpu.bitcast(pltpu.bitcast(kr, jnp.int32) | jnp.tile(zm, (NVG, 1)), F32)
                        build_kb(krz, 1 - par, (2 * u, 2 * u + 1))
            if h2 is not None:
                o = acc / acc[lrow:lrow + 1, :]
                pltpu.store(ot_ref.at[pl.ds(w0, VROWS), cols], o, mask=ovalid)

    def last_heads(u):
        base = pl.multiple_of(u * RB, RB)
        half = [pl.ds(base + i * 128, 128) for i in range(2)]
        o = [ot_ref[0:512, r].T.astype(BF16) for r in half]
        pieces = [(i, n, k) for k in range(2) for i in range(2) for n in range(NTILE)]

        def piece(j):
            i, n, k = pieces[j]
            x_ref[half[i], n * 128:(n + 1) * 128] += _dot(
                o[i][:, k * 256:(k + 1) * 256], wbo_ref[k * 256:(k + 1) * 256, n * 128:(n + 1) * 128])
        slots = tuple(2 * t for t in (0, 2, 4, 7, 9, 11, 14, 16, 18, 21, 23, 25, 28, 30))

        def extra(first):
            def f(ui, c):
                step = first + ui * NC + c
                if step in slots:
                    piece(slots.index(step))
            return f
        attn(None, H - 2, 0, extra(0), blocks=[2 * u, 2 * u + 1])
        attn(None, H - 1, 1, extra(2 * NC), blocks=[2 * u, 2 * u + 1])
        for j in range(len(slots), len(pieces)):
            piece(j)
        rows = rows_of(u)
        xb = x_ref[rows, :] + _dot(ot_ref[512:D, rows].T.astype(BF16), wbo_ref[512:D, :])
        x_ref[rows, :] = xb
        xin_ref[rows, :] = xb.astype(BF16)
        out_copy(u).start()

    cp_wak.start()
    x_copy(0).start()
    cp_waq.start()
    x_copy(1).start()
    x_copy(2).start()
    g_ref[...] = jnp.zeros(g_ref.shape, F32)
    zp_ref[...] = jnp.zeros(zp_ref.shape, F32)
    zv_ref[...] = jnp.zeros(zv_ref.shape, jnp.int32)
    zero_ref[0, 0] = 0
    cp_wak.wait()
    for b in range(3, NB):
        x_copy(b).start()
    cp_wav.start()
    cp_wao.start()
    cp_wb.start()
    cp_wbo.start()
    wat_ref[0:D, :] = wa_ref[:, D:2 * D].astype(F32).T.astype(BF16)
    x_copy(0).wait()
    x0 = xin_ref[rows_of(0), :].astype(F32)
    x_ref[rows_of(0), :] = x0
    xn_ref[...] = _layernorm(x0)
    cp_waq.wait()
    wat_ref[D:2 * D, :] = wa_ref[:, 0:D].astype(F32).T.astype(BF16)

    def two_layers(it, c):
        first = it == 0

        def load_x(b):
            rows = rows_of(b)
            xb = jnp.where(first, xin_ref[rows, :].astype(F32), x_ref[rows, :])
            x_ref[rows, :] = xb
            return _layernorm(xb)

        def a1_body(j, c):
            @pl.when(first)
            def _():
                x_copy(2 * j + 1).wait()

                @pl.when(j < NIT - 1)
                def _():
                    x_copy(2 * j + 2).wait()
            a1_pair(j, load_x)
            return c
        lax.fori_loop(0, NIT, a1_body, 0)

        @pl.when(first)
        def _():
            cp_wav.wait()
            cp_wao.wait()
            cp_wb.wait()
            cp_wbo.wait()

        @pl.when(jnp.logical_not(first))
        def _():
            for b in range(NB):
                out_copy(b).wait()

        wbt_ref[0:D, :] = wb_ref[:, 0:D].astype(F32).T.astype(BF16)
        wbt_ref[D:2 * D, :] = wb_ref[:, 2 * D:3 * D].astype(F32).T.astype(BF16)
        xn_ref[...] = _layernorm(a3_x(0, a2()))

        def a3_b1(b, c):
            y = a3_y(b + 1)
            b1_k(b, xn_ref[...])
            xn_next = _layernorm(a3_x(b + 1, y))
            b1_qv(b, xn_ref[...])
            xn_ref[...] = xn_next
            return c
        lax.fori_loop(0, NB - 1, a3_b1, 0)
        b1_k(NB - 1, xn_ref[...])
        b1_qv(NB - 1, xn_ref[...])

        def first_scores(h, c):
            build_kb(vpu_keys(2), 0, range(DH))
            attn(h, None, h)
            return c
        lax.fori_loop(0, 2, first_scores, 0)

        def body(i, c):
            pace = []
            attn(2 * i + 2, 2 * i, 0, vpu=True, pace=pace)
            attn(2 * i + 3, 2 * i + 1, 1, vpu=True, pace=pace)
            return c
        lax.fori_loop(0, H // 2 - 1, body, 0)

        def tail(j, c):
            last_heads(2 * j)
            last_heads(2 * j + 1)
            return c
        lax.fori_loop(0, NIT, tail, 0)

        @pl.when(first)
        def _():
            xn_ref[...] = _layernorm(x_ref[rows_of(0), :])
        return c
    lax.fori_loop(0, 2, two_layers, 0)
    for b in range(NB):
        out_copy(b).wait()


@jax.jit
def pallas_interleave_layers__linear_attn_block__mha_block__prompt_kernel(
    A_x: jax.Array,
    A_wqkv: jax.Array,
    A_wo: jax.Array,
    B_x: jax.Array,
    B_wqkv: jax.Array,
    B_wo: jax.Array,
):
    del B_x
    x = A_x.reshape(S, D)
    any_spec = pl.BlockSpec(memory_space=pl.ANY)
    out = pl.pallas_call(
        _kernel,
        out_shape=jax.ShapeDtypeStruct((S, D), BF16),
        in_specs=[any_spec] * 5,
        out_specs=any_spec,
        scratch_shapes=[
            pltpu.VMEM((S, D), BF16),
            pltpu.VMEM((D, 3 * D), BF16),
            pltpu.VMEM((D, D), BF16),
            pltpu.VMEM((D, 3 * D), BF16),
            pltpu.VMEM((D, D), BF16),
            pltpu.SemaphoreType.DMA((NB + 6,)),
            pltpu.VMEM((S, D), F32),
            pltpu.VMEM((RB, D), BF16),
            pltpu.VMEM((2 * D, D), BF16),
            pltpu.VMEM((2 * D, D), BF16),
            pltpu.VMEM((D, S), F32),
            pltpu.VMEM((D, D), F32),
            pltpu.VMEM((D, 128), F32),
            pltpu.VMEM((D, D), BF16),
            pltpu.VMEM((H, D), F32),
            pltpu.VMEM((NQ, D, TQ), F32),
            pltpu.VMEM((2 * NTILE - 1, S, 128), F32),
            pltpu.VMEM((D, S), F32),
            pltpu.VMEM((D, S), F32),
            pltpu.VMEM((2, NQ, S, TQ), F32),
            pltpu.VMEM((2, NQ, 8, TQ), F32),
            pltpu.VMEM((NQ, DH, 8, TQ), F32),
            pltpu.VMEM((NQ, DH, 8, TQ), F32),
            pltpu.VMEM((NVG, DH, 8, TQ), F32),
            pltpu.VMEM((NVG, DH, 8, TQ), F32),
            pltpu.VMEM((8, TQ), jnp.int32),
            pltpu.SMEM((1, 1), jnp.int32),
        ],
        compiler_params=pltpu.CompilerParams(vmem_limit_bytes=110 * 1024 * 1024),
    )(x, A_wqkv, A_wo, B_wqkv, B_wo)
    return out.reshape(1, S, D)
```

```python
import jax
import jax.numpy as jnp
from jax import lax
import jax.experimental.pallas as pl
import jax.experimental.pallas.tpu as pltpu

S = 2048
D = 640
H = 32
DH = 20
NTILE = D // 128
RB = 256
NB = S // RB
NIT = NB // 2
TQ = 128
TK = 128
NQ = S // TQ
NC = S // TK
VR = 8
PACE = 3
PACE_FIRST = 5
TAIL_FIRST = 6
TAIL_LEFT = 10
VROWS = 24
KV_ROWS = ((0, 144), (112, 272), (240, 400), (368, 528), (496, 640))

LOG2E = 1.4426950408889634
QSCALE = (DH ** -0.5) * LOG2E

F32 = jnp.float32
BF16 = jnp.bfloat16
_NT = (((1,), (1,)), ((), ()))


def _dot(a, b):
    return jnp.dot(a, b, preferred_element_type=F32)


def _dot_nt(a, b):
    return lax.dot_general(a, b, _NT, preferred_element_type=F32)


def _layernorm(xb):
    m = jnp.mean(xb, axis=-1, keepdims=True)
    xc = xb - m
    v = jnp.mean(xc * xc, axis=-1, keepdims=True)
    return (xc * lax.rsqrt(v + 1e-5)).astype(BF16)


def _phi(t):
    return jnp.where(t > 0, t + 1.0, jnp.exp(t)) + 1e-6


def _kernel(x_hbm, wa_hbm, wao_hbm, wb_hbm, wbo_hbm, out_hbm,
            xin_ref, wa_ref, wao_ref, wb_ref, wbo_ref, sems,
            x_ref, xn_ref, wat_ref, wbt_ref, pq_ref, g_ref, zp_ref, m_ref, zh_ref,
            qt_ref, k_ref, vt_ref, ot_ref, s_ref, mx_ref,
            qb0_ref, qb1_ref, kb0_ref, kb1_ref, kf_ref, qf_ref, zv_ref, zero_ref):
    qb_refs = (qb0_ref, qb1_ref)
    kb_refs = (kb0_ref, kb1_ref)

    def rows_of(b):
        if isinstance(b, int):
            return slice(b * RB, (b + 1) * RB)
        return pl.ds(pl.multiple_of(b * RB, RB), RB)

    def x_copy(b):
        return pltpu.make_async_copy(x_hbm.at[rows_of(b), :], xin_ref.at[rows_of(b), :], sems.at[b])

    def out_copy(b):
        return pltpu.make_async_copy(xin_ref.at[rows_of(b), :], out_hbm.at[rows_of(b), :], sems.at[b])

    cp_wak = pltpu.make_async_copy(wa_hbm.at[:, pl.ds(D, D)], wa_ref.at[:, pl.ds(D, D)], sems.at[NB])
    cp_waq = pltpu.make_async_copy(wa_hbm.at[:, pl.ds(0, D)], wa_ref.at[:, pl.ds(0, D)], sems.at[NB + 1])
    cp_wav = pltpu.make_async_copy(wa_hbm.at[:, pl.ds(2 * D, D)], wa_ref.at[:, pl.ds(2 * D, D)],
                                   sems.at[NB + 2])
    cp_wao = pltpu.make_async_copy(wao_hbm, wao_ref, sems.at[NB + 3])
    cp_wb = pltpu.make_async_copy(wb_hbm, wb_ref, sems.at[NB + 4])
    cp_wbo = pltpu.make_async_copy(wbo_hbm, wbo_ref, sems.at[NB + 5])

    def a1_stage(b, xn):
        pkt = _phi(_dot_nt(wat_ref[0:D, :], xn))
        pq_ref[:, rows_of(b)] = _phi(_dot_nt(wat_ref[D:2 * D, :], xn))
        zp = pkt[:, 0:128]
        for t in range(1, RB // 128):
            zp = zp + pkt[:, t * 128:(t + 1) * 128]
        return zp, _dot(pkt.astype(BF16), xn)

    def a1_pair(j, ln_of):
        xn_b = ln_of(2 * j + 1)
        zp0, g0 = a1_stage(2 * j, xn_ref[...])
        xn_ref[...] = ln_of(jnp.minimum(2 * j + 2, NB - 1))
        zp1, g1 = a1_stage(2 * j + 1, xn_b)
        zp_ref[...] += zp0 + zp1
        g_ref[...] += g0 + g1

    def a2():
        z = jnp.sum(zp_ref[...].T, axis=0, keepdims=True)
        hj = lax.broadcasted_iota(jnp.int32, (H, D), 0) * DH
        cd = lax.broadcasted_iota(jnp.int32, (H, D), 1)
        zh_ref[...] = jnp.where((cd >= hj) & (cd < hj + DH), z, 0.0)
        kvm = []
        for t, (lo, hi) in enumerate(KV_ROWS):
            n = hi - lo
            kv = _dot(g_ref[lo:hi, :].astype(BF16), wa_ref[:, 2 * D + t * 128:2 * D + (t + 1) * 128])
            rd = lax.broadcasted_iota(jnp.int32, (n, 128), 0) + lo
            ce = lax.broadcasted_iota(jnp.int32, (n, 128), 1) + t * 128
            h0 = ((rd * 3277) >> 16) * DH
            kvm.append(jnp.where((ce >= h0) & (ce < h0 + DH), kv, 0.0).astype(BF16))
        y0 = a3_y(0)
        mt = [_dot(kvm[t], wao_ref[t * 128:(t + 1) * 128, :]) for t in range(NTILE)]
        for t, (lo, hi) in enumerate(KV_ROWS):
            a = KV_ROWS[t - 1][1] if t > 0 else lo
            b = KV_ROWS[t + 1][0] if t + 1 < NTILE else hi
            m_ref[a:b, :] = mt[t][a - lo:b - lo, :].astype(BF16)
            if b < hi:
                m_ref[b:hi, :] = (mt[t][b - lo:, :] + mt[t + 1][0:hi - b, :]).astype(BF16)
        g_ref[...] = jnp.zeros(g_ref.shape, F32)
        zp_ref[...] = jnp.zeros(zp_ref.shape, F32)
        return y0

    def a3_y(b):
        rows = rows_of(b)
        r = 1.0 / (_dot(zh_ref[...], pq_ref[:, rows]) + 1e-6)
        sub = lax.broadcasted_iota(jnp.int32, (8, RB), 0)
        pieces = []
        for j in range(H // 2):
            ra = jnp.broadcast_to(r[2 * j:2 * j + 1, :], (8, RB))
            rb = jnp.broadcast_to(r[2 * j + 1:2 * j + 2, :], (8, RB))
            pieces += [ra, ra, jnp.where(sub < 4, ra, rb), rb, rb]
        return (pq_ref[:, rows] * jnp.concatenate(pieces, axis=0)).T.astype(BF16)

    def a3_x(b, y):
        xb = x_ref[rows_of(b), :] + _dot(y, m_ref[...])
        x_ref[rows_of(b), :] = xb
        return xb

    def b1_k(b, xn):
        rows = rows_of(b)
        k = _dot(xn, wb_ref[:, D:2 * D])
        lane = lax.broadcasted_iota(jnp.int32, (RB, 128), 1)
        for t in range(NTILE):
            k_ref[t, rows, :] = k[:, t * 128:(t + 1) * 128]
        for t in range(NTILE - 1):
            k_ref[NTILE + t, rows, :] = jnp.where(
                lane >= 64, k[:, t * 128:(t + 1) * 128],
                k[:, (t + 1) * 128:(t + 2) * 128])

        for i in range(RB // TK):
            c = b * (RB // TK) + i
            kr = k[i * TK:i * TK + VR, 0:128]
            for d in range(2 * DH):
                kf_ref[d // DH, c, d % DH] = jnp.broadcast_to(kr[:, d:d + 1], (VR, TQ))
            for dd in range(DH):
                kb_refs[0][c, dd] = jnp.broadcast_to(kr[:, 2 * DH + dd:2 * DH + dd + 1], (VR, TQ))

    def b1_qv(b, xn):
        rows = rows_of(b)
        qvt = _dot_nt(wbt_ref[...], xn)
        for i in range(RB // TQ):
            qs = qvt[0:D, i * TQ:(i + 1) * TQ] * QSCALE
            qt_ref[b * (RB // TQ) + i] = qs
            for d in range(2 * DH):
                qf_ref[d // DH, b * (RB // TQ) + i, d % DH] = jnp.broadcast_to(qs[d:d + 1, :], (8, TQ))
            for par in range(2):
                for dd in range(DH):
                    r = (2 + par) * DH + dd
                    qb_refs[par][b * (RB // TQ) + i, dd] = jnp.broadcast_to(qs[r:r + 1, :], (8, TQ))
        vt_ref[:, rows] = qvt[D:2 * D, :]

    def cols_of(u):
        if isinstance(u, int):
            return slice(u * TQ, (u + 1) * TQ)
        return pl.ds(pl.multiple_of(u * TQ, TQ), TQ)

    def build_qb(h, par, u):
        win = qt_ref[u, pl.ds(pl.multiple_of(h * DH - 4 * par, 8), VROWS), :]
        for dd in range(DH):
            r = 4 * par + dd
            qb_refs[par][u, dd] = jnp.broadcast_to(win[r:r + 1, :], (8, TQ))

    def vpu_keys(h):
        d0 = h * DH
        lo = d0 & 127
        ktile = jnp.where(lo > 128 - DH, NTILE + (d0 >> 7), d0 >> 7)
        rows = jnp.concatenate([k_ref[ktile, c * TK:c * TK + VR, :] for c in range(NC)], axis=0)
        return pltpu.roll(rows, (128 - lo) & 127, axis=1)

    def build_kb(kr, par, ds):
        for dd in ds:
            kbd = jnp.broadcast_to(kr[:, dd:dd + 1], (NC * VR, TQ))
            for c in range(NC):
                kb_refs[par][c, dd + zero_ref[0, 0]] = kbd[c * VR:(c + 1) * VR, :]

    def attn(h1, h2, par, extra=None, blocks=None, vpu=False, pace=None, outs=None, first=False):
        if h1 is not None:
            d0 = h1 * DH
            t = d0 >> 7
            lo = d0 & 127
            ktile = jnp.where(lo > 128 - DH, NTILE + t, t)
            t_hi = pl.multiple_of(t * 128, 128)
            t_lo = pl.multiple_of(jnp.minimum(t + 1, NTILE - 1) * 128, 128)
            r = lax.broadcasted_iota(jnp.int32, (128, TQ), 0)
            head_bits = jnp.where(((r - lo) & 127) < DH, -1, zero_ref[0, 0])
            upper = r >= lo
            lag = PACE_FIRST if first else PACE
            if vpu:
                kr = vpu_keys(jnp.minimum(h1 + 1, H - 1))
        if h2 is not None:
            off = 4 * par
            w0 = pl.multiple_of(h2 * DH - off, 8)
            rv = lax.broadcasted_iota(jnp.int32, (VROWS, S), 0)
            vt = jnp.where((rv >= off) & (rv < off + DH), vt_ref[pl.ds(w0, VROWS), :], 1.0)
            ro = lax.broadcasted_iota(jnp.int32, (VROWS, TQ), 0)
            ovalid = (ro >= off) & (ro < off + DH)
            lrow = DH if par == 0 else 0
        for ui, u in enumerate(range(NQ) if blocks is None else blocks):
            cols = cols_of(u)
            if h1 is not None:
                qw = jnp.where(upper, qt_ref[u, pl.ds(t_hi, 128), :], qt_ref[u, pl.ds(t_lo, 128), :])
                qw = pltpu.bitcast(pltpu.bitcast(qw, jnp.int32) & head_bits, F32)
            if h2 is not None:
                m2 = mx_ref[par, u]
            m = None
            acc = None
            for c in range(NC):
                ks = slice(c * TK, (c + 1) * TK)
                if h1 is not None:
                    sv = None
                    for dd in range(DH):
                        kb = kf_ref[h1, c, dd] if first else kb_refs[par][c, dd]
                        if dd == 0 and len(pace) >= lag:
                            zs = pltpu.bitcast(pace[-lag][0:8, :], jnp.int32) & zv_ref[...]
                            kb = pltpu.bitcast(pltpu.bitcast(kb, jnp.int32) | zs, F32)
                        tt = kb * (qf_ref[h1, u, dd] if first else qb_refs[par][u, dd])
                        sv = tt if sv is None else sv + tt
                if h2 is not None:
                    s = s_ref[par, u, ks, :]
                    p = jnp.exp2(s.reshape(TK // 8, 8, TQ) - m2[None]).reshape(TK, TQ)
                    d = _dot(vt[:, ks], p)
                    acc = d if acc is None else acc + d
                if h1 is not None:
                    s = _dot(k_ref[ktile, c * TK + VR:(c + 1) * TK, :], qw)
                    pace.append(s)
                    s = jnp.concatenate([sv, s], axis=0)
                    s_ref[par, u, ks, :] = s
                    mc = jnp.max(s.reshape(TK // 8, 8, TQ), axis=0)
                    m = mc if m is None else jnp.maximum(m, mc)
                if extra is not None:
                    extra(ui, c)
            if h1 is not None:
                m = jnp.max(m, axis=0, keepdims=True)
                mx_ref[par, u] = jnp.broadcast_to(m, (8, TQ))
                if vpu:
                    build_qb(jnp.minimum(h1 + 2, H - 2 + par), par, u)
                    if 2 * u < DH:
                        zm = pltpu.bitcast(jnp.broadcast_to(m, (8, TQ)), jnp.int32) & zv_ref[...]
                        krz = pltpu.bitcast(pltpu.bitcast(kr, jnp.int32) | jnp.tile(zm, (NC, 1)), F32)
                        build_kb(krz, 1 - par, (2 * u, 2 * u + 1))
            if h2 is not None:
                o = acc / acc[lrow:lrow + 1, :]
                if outs is None:
                    pltpu.store(ot_ref.at[pl.ds(w0, VROWS), cols], o, mask=ovalid)
                else:
                    outs.append(o)

    def last_heads(j):
        base = pl.multiple_of(j * 2 * RB, 2 * RB)
        quarter = [pl.ds(base + i * 128, 128) for i in range(4)]
        o = [ot_ref[0:512, r].T.astype(BF16) for r in quarter]

        outs = ([], [])

        def piece(i, n, k):
            x_ref[quarter[i], n * 128:(n + 1) * 128] += _dot(
                o[i][:, k * 256:(k + 1) * 256], wbo_ref[k * 256:(k + 1) * 256, n * 128:(n + 1) * 128])

        def finish(i):
            r = quarter[i]
            oa, ob = outs[0][i], outs[1][i]
            sub = lax.broadcasted_iota(jnp.int32, (8, TQ), 0)
            last = jnp.concatenate([ot_ref[512:D - 2 * DH, r], oa[0:16, :],
                                    jnp.where(sub < 4, oa[16:24, :], ob[0:8, :]), ob[8:24, :]], axis=0)
            xb = x_ref[r, :] + _dot(last.T.astype(BF16), wbo_ref[512:D, :])
            x_ref[r, :] = xb
            xin_ref[r, :] = xb.astype(BF16)
            if i % 2 == 1:
                out_copy(2 * j + i // 2).start()

        def pieces(b):
            return [(piece, (i, n, k)) for k in range(2) for i in (2 * b, 2 * b + 1) for n in range(NTILE)]
        jobs = pieces(0) + pieces(1)[:4] + [(finish, (0,)), (finish, (1,))] + pieces(1)[4:]
        jobs += [(finish, (2,)), (finish, (3,))]
        n_in = len(jobs) - TAIL_LEFT
        slots = [TAIL_FIRST + (t * (8 * NC - TAIL_FIRST)) // n_in for t in range(n_in)]

        def extra(first):
            def f(ui, c):
                step = first + ui * NC + c
                while step in slots:
                    fn, args = jobs[slots.index(step)]
                    slots[slots.index(step)] = -1
                    fn(*args)
            return f
        for b in range(2):
            blocks = [4 * j + 2 * b, 4 * j + 2 * b + 1]
            attn(None, H - 2, 0, extra(4 * b * NC), blocks=blocks, outs=outs[0])
            attn(None, H - 1, 1, extra((4 * b + 2) * NC), blocks=blocks, outs=outs[1])
        for fn, args in jobs[n_in:]:
            fn(*args)

    cp_wak.start()
    x_copy(0).start()
    cp_waq.start()
    x_copy(1).start()
    x_copy(2).start()
    g_ref[...] = jnp.zeros(g_ref.shape, F32)
    zp_ref[...] = jnp.zeros(zp_ref.shape, F32)
    zv_ref[...] = jnp.zeros(zv_ref.shape, jnp.int32)
    zero_ref[0, 0] = 0
    cp_wak.wait()
    for b in range(3, NB):
        x_copy(b).start()
    cp_wav.start()
    cp_wao.start()
    cp_wb.start()
    cp_wbo.start()
    wat_ref[0:D, :] = wa_ref[:, D:2 * D].astype(F32).T.astype(BF16)
    x_copy(0).wait()
    x0 = xin_ref[rows_of(0), :].astype(F32)
    x_ref[rows_of(0), :] = x0
    xn_ref[...] = _layernorm(x0)
    cp_waq.wait()
    wat_ref[D:2 * D, :] = wa_ref[:, 0:D].astype(F32).T.astype(BF16)

    def two_layers(it, c):
        first = it == 0

        def load_x(b):
            rows = rows_of(b)
            xb = jnp.where(first, xin_ref[rows, :].astype(F32), x_ref[rows, :])
            x_ref[rows, :] = xb
            return _layernorm(xb)

        def a1_body(j, c):
            @pl.when(first)
            def _():
                x_copy(2 * j + 1).wait()

                @pl.when(j < NIT - 1)
                def _():
                    x_copy(2 * j + 2).wait()
            a1_pair(j, load_x)
            return c
        lax.fori_loop(0, NIT, a1_body, 0)

        @pl.when(first)
        def _():
            cp_wav.wait()
            cp_wao.wait()
            cp_wb.wait()
            cp_wbo.wait()

        @pl.when(jnp.logical_not(first))
        def _():
            for b in range(NB):
                out_copy(b).wait()

        wbt_ref[0:D, :] = wb_ref[:, 0:D].astype(F32).T.astype(BF16)
        wbt_ref[D:2 * D, :] = wb_ref[:, 2 * D:3 * D].astype(F32).T.astype(BF16)
        xn_ref[...] = _layernorm(a3_x(0, a2()))

        def a3_b1(b, c):
            y = a3_y(b + 1)
            b1_k(b, xn_ref[...])
            xn_next = _layernorm(a3_x(b + 1, y))
            b1_qv(b, xn_ref[...])
            xn_ref[...] = xn_next
            return c
        lax.fori_loop(0, NB - 1, a3_b1, 0)
        b1_k(NB - 1, xn_ref[...])
        b1_qv(NB - 1, xn_ref[...])

        def first_scores(h, c):
            attn(h, None, h, pace=[], first=True)
            return c
        lax.fori_loop(0, 2, first_scores, 0)

        def body(i, c):
            pace = []
            attn(2 * i + 2, 2 * i, 0, vpu=True, pace=pace)
            attn(2 * i + 3, 2 * i + 1, 1, vpu=True, pace=pace)
            return c
        lax.fori_loop(0, H // 2 - 1, body, 0)

        def tail(j, c):
            last_heads(j)
            return c
        lax.fori_loop(0, NIT, tail, 0)

        @pl.when(first)
        def _():
            xn_ref[...] = _layernorm(x_ref[rows_of(0), :])
        return c
    lax.fori_loop(0, 2, two_layers, 0)
    for b in range(NB):
        out_copy(b).wait()


@jax.jit
def pallas_interleave_layers__linear_attn_block__mha_block__prompt_kernel(
    A_x: jax.Array,
    A_wqkv: jax.Array,
    A_wo: jax.Array,
    B_x: jax.Array,
    B_wqkv: jax.Array,
    B_wo: jax.Array,
):
    del B_x
    x = A_x.reshape(S, D)
    any_spec = pl.BlockSpec(memory_space=pl.ANY)
    out = pl.pallas_call(
        _kernel,
        out_shape=jax.ShapeDtypeStruct((S, D), BF16),
        in_specs=[any_spec] * 5,
        out_specs=any_spec,
        scratch_shapes=[
            pltpu.VMEM((S, D), BF16),
            pltpu.VMEM((D, 3 * D), BF16),
            pltpu.VMEM((D, D), BF16),
            pltpu.VMEM((D, 3 * D), BF16),
            pltpu.VMEM((D, D), BF16),
            pltpu.SemaphoreType.DMA((NB + 6,)),
            pltpu.VMEM((S, D), F32),
            pltpu.VMEM((RB, D), BF16),
            pltpu.VMEM((2 * D, D), BF16),
            pltpu.VMEM((2 * D, D), BF16),
            pltpu.VMEM((D, S), F32),
            pltpu.VMEM((D, D), F32),
            pltpu.VMEM((D, 128), F32),
            pltpu.VMEM((D, D), BF16),
            pltpu.VMEM((H, D), F32),
            pltpu.VMEM((NQ, D, TQ), F32),
            pltpu.VMEM((2 * NTILE - 1, S, 128), F32),
            pltpu.VMEM((D, S), F32),
            pltpu.VMEM((D, S), F32),
            pltpu.VMEM((2, NQ, S, TQ), F32),
            pltpu.VMEM((2, NQ, 8, TQ), F32),
            pltpu.VMEM((NQ, DH, 8, TQ), F32),
            pltpu.VMEM((NQ, DH, 8, TQ), F32),
            pltpu.VMEM((NC, DH, VR, TQ), F32),
            pltpu.VMEM((NC, DH, VR, TQ), F32),
            pltpu.VMEM((2, NC, DH, VR, TQ), F32),
            pltpu.VMEM((2, NQ, DH, 8, TQ), F32),
            pltpu.VMEM((8, TQ), jnp.int32),
            pltpu.SMEM((1, 1), jnp.int32),
        ],
        compiler_params=pltpu.CompilerParams(vmem_limit_bytes=110 * 1024 * 1024),
    )(x, A_wqkv, A_wo, B_wqkv, B_wo)
    return out.reshape(1, S, D)
```

```python
import jax
import jax.numpy as jnp
from jax import lax
import jax.experimental.pallas as pl
import jax.experimental.pallas.tpu as pltpu

S = 2048
D = 640
H = 32
DH = 20
NTILE = D // 128
RB = 256
NB = S // RB
NIT = NB // 2
TQ = 128
TK = 128
NQ = S // TQ
NC = S // TK
VR = 8
PACE = 5
PACE_FIRST = 5
TAIL_FIRST = 6
TAIL_LEFT = 10
VROWS = 24
KV_ROWS = ((0, 144), (112, 272), (240, 400), (368, 528), (496, 640))

LOG2E = 1.4426950408889634
QSCALE = (DH ** -0.5) * LOG2E

F32 = jnp.float32
BF16 = jnp.bfloat16
_NT = (((1,), (1,)), ((), ()))


def _dot(a, b):
    return jnp.dot(a, b, preferred_element_type=F32)


def _dot_nt(a, b):
    return lax.dot_general(a, b, _NT, preferred_element_type=F32)


def _layernorm(xb):
    m = jnp.mean(xb, axis=-1, keepdims=True)
    xc = xb - m
    v = jnp.mean(xc * xc, axis=-1, keepdims=True)
    return (xc * lax.rsqrt(v + 1e-5)).astype(BF16)


def _phi(t):
    return jnp.where(t > 0, t + 1.0, jnp.exp(t)) + 1e-6


def _kernel(x_hbm, wa_hbm, wao_hbm, wb_hbm, wbo_hbm, out_hbm,
            xin_ref, wa_ref, wao_ref, wb_ref, wbo_ref, sems,
            x_ref, xn_ref, wat_ref, wbt_ref, pq_ref, g_ref, zp_ref, m_ref, zh_ref,
            qt_ref, k_ref, vt_ref, ot_ref, s_ref, mx_ref,
            qb0_ref, qb1_ref, kb0_ref, kb1_ref, kf_ref, qf_ref, zv_ref, zero_ref):
    qb_refs = (qb0_ref, qb1_ref)
    kb_refs = (kb0_ref, kb1_ref)

    def rows_of(b):
        if isinstance(b, int):
            return slice(b * RB, (b + 1) * RB)
        return pl.ds(pl.multiple_of(b * RB, RB), RB)

    def x_copy(b):
        return pltpu.make_async_copy(x_hbm.at[rows_of(b), :], xin_ref.at[rows_of(b), :], sems.at[b])

    def out_copy(b):
        return pltpu.make_async_copy(xin_ref.at[rows_of(b), :], out_hbm.at[rows_of(b), :], sems.at[b])

    cp_wak = pltpu.make_async_copy(wa_hbm.at[:, pl.ds(D, D)], wa_ref.at[:, pl.ds(D, D)], sems.at[NB])
    cp_waq = pltpu.make_async_copy(wa_hbm.at[:, pl.ds(0, D)], wa_ref.at[:, pl.ds(0, D)], sems.at[NB + 1])
    cp_wav = pltpu.make_async_copy(wa_hbm.at[:, pl.ds(2 * D, D)], wa_ref.at[:, pl.ds(2 * D, D)],
                                   sems.at[NB + 2])
    cp_wao = pltpu.make_async_copy(wao_hbm, wao_ref, sems.at[NB + 3])
    cp_wb = pltpu.make_async_copy(wb_hbm, wb_ref, sems.at[NB + 4])
    cp_wbo = pltpu.make_async_copy(wbo_hbm, wbo_ref, sems.at[NB + 5])

    def a1_stage(b, xn):
        pkt = _phi(_dot_nt(wat_ref[0:D, :], xn))
        pq_ref[:, rows_of(b)] = _phi(_dot_nt(wat_ref[D:2 * D, :], xn))
        zp = pkt[:, 0:128]
        for t in range(1, RB // 128):
            zp = zp + pkt[:, t * 128:(t + 1) * 128]
        return zp, _dot(pkt.astype(BF16), xn)

    def a1_pair(j, ln_of):
        xn_b = ln_of(2 * j + 1)
        zp0, g0 = a1_stage(2 * j, xn_ref[...])
        xn_ref[...] = ln_of(jnp.minimum(2 * j + 2, NB - 1))
        zp1, g1 = a1_stage(2 * j + 1, xn_b)
        zp_ref[...] += zp0 + zp1
        g_ref[...] += g0 + g1

    def a2():
        z = jnp.sum(zp_ref[...].T, axis=0, keepdims=True)
        hj = lax.broadcasted_iota(jnp.int32, (H, D), 0) * DH
        cd = lax.broadcasted_iota(jnp.int32, (H, D), 1)
        zh_ref[...] = jnp.where((cd >= hj) & (cd < hj + DH), z, 0.0)
        kvm = []
        for t, (lo, hi) in enumerate(KV_ROWS):
            n = hi - lo
            kv = _dot(g_ref[lo:hi, :].astype(BF16), wa_ref[:, 2 * D + t * 128:2 * D + (t + 1) * 128])
            rd = lax.broadcasted_iota(jnp.int32, (n, 128), 0) + lo
            ce = lax.broadcasted_iota(jnp.int32, (n, 128), 1) + t * 128
            h0 = ((rd * 3277) >> 16) * DH
            kvm.append(jnp.where((ce >= h0) & (ce < h0 + DH), kv, 0.0).astype(BF16))
        y0 = a3_y(0)
        mt = [_dot(kvm[t], wao_ref[t * 128:(t + 1) * 128, :]) for t in range(NTILE)]
        for t, (lo, hi) in enumerate(KV_ROWS):
            a = KV_ROWS[t - 1][1] if t > 0 else lo
            b = KV_ROWS[t + 1][0] if t + 1 < NTILE else hi
            m_ref[a:b, :] = mt[t][a - lo:b - lo, :].astype(BF16)
            if b < hi:
                m_ref[b:hi, :] = (mt[t][b - lo:, :] + mt[t + 1][0:hi - b, :]).astype(BF16)
        g_ref[...] = jnp.zeros(g_ref.shape, F32)
        zp_ref[...] = jnp.zeros(zp_ref.shape, F32)
        return y0

    def a3_y(b):
        rows = rows_of(b)
        r = 1.0 / (_dot(zh_ref[...], pq_ref[:, rows]) + 1e-6)
        sub = lax.broadcasted_iota(jnp.int32, (8, RB), 0)
        pieces = []
        for j in range(H // 2):
            ra = jnp.broadcast_to(r[2 * j:2 * j + 1, :], (8, RB))
            rb = jnp.broadcast_to(r[2 * j + 1:2 * j + 2, :], (8, RB))
            pieces += [ra, ra, jnp.where(sub < 4, ra, rb), rb, rb]
        return (pq_ref[:, rows] * jnp.concatenate(pieces, axis=0)).T.astype(BF16)

    def a3_x(b, y):
        xb = x_ref[rows_of(b), :] + _dot(y, m_ref[...])
        x_ref[rows_of(b), :] = xb
        return xb

    def b1_k(b, xn):
        rows = rows_of(b)
        k = _dot(xn, wb_ref[:, D:2 * D])
        lane = lax.broadcasted_iota(jnp.int32, (RB, 128), 1)
        for t in range(NTILE):
            k_ref[t, rows, :] = k[:, t * 128:(t + 1) * 128]
        for t in range(NTILE - 1):
            k_ref[NTILE + t, rows, :] = jnp.where(
                lane >= 64, k[:, t * 128:(t + 1) * 128],
                k[:, (t + 1) * 128:(t + 2) * 128])

        for i in range(RB // TK):
            c = b * (RB // TK) + i
            kr = k[i * TK:i * TK + VR, 0:128]
            for d in range(2 * DH):
                kf_ref[d // DH, c, d % DH] = jnp.broadcast_to(kr[:, d:d + 1], (VR, TQ))
            for dd in range(DH):
                kb_refs[0][c, dd] = jnp.broadcast_to(kr[:, 2 * DH + dd:2 * DH + dd + 1], (VR, TQ))

    def b1_qv(b, xn):
        rows = rows_of(b)
        qvt = _dot_nt(wbt_ref[...], xn)
        for i in range(RB // TQ):
            qs = qvt[0:D, i * TQ:(i + 1) * TQ] * QSCALE
            qt_ref[b * (RB // TQ) + i] = qs
            for d in range(2 * DH):
                qf_ref[d // DH, b * (RB // TQ) + i, d % DH] = jnp.broadcast_to(qs[d:d + 1, :], (8, TQ))
            for par in range(2):
                for dd in range(DH):
                    r = (2 + par) * DH + dd
                    qb_refs[par][b * (RB // TQ) + i, dd] = jnp.broadcast_to(qs[r:r + 1, :], (8, TQ))
        vt_ref[:, rows] = qvt[D:2 * D, :]

    def cols_of(u):
        if isinstance(u, int):
            return slice(u * TQ, (u + 1) * TQ)
        return pl.ds(pl.multiple_of(u * TQ, TQ), TQ)

    def build_qb(h, par, u):
        win = qt_ref[u, pl.ds(pl.multiple_of(h * DH - 4 * par, 8), VROWS), :]
        for dd in range(DH):
            r = 4 * par + dd
            qb_refs[par][u, dd] = jnp.broadcast_to(win[r:r + 1, :], (8, TQ))

    def vpu_keys(h):
        d0 = h * DH
        lo = d0 & 127
        ktile = jnp.where(lo > 128 - DH, NTILE + (d0 >> 7), d0 >> 7)
        rows = jnp.concatenate([k_ref[ktile, c * TK:c * TK + VR, :] for c in range(NC)], axis=0)
        return pltpu.roll(rows, (128 - lo) & 127, axis=1)

    def build_kb(kr, par, ds):
        for dd in ds:
            kbd = jnp.broadcast_to(kr[:, dd:dd + 1], (NC * VR, TQ))
            kb_refs[par][:, dd + zero_ref[0, 0]] = kbd.reshape(NC, VR, TQ)

    def attn(h1, h2, par, extra=None, blocks=None, vpu=False, pace=None, outs=None, first=False):
        if h1 is not None:
            d0 = h1 * DH
            t = d0 >> 7
            lo = d0 & 127
            ktile = jnp.where(lo > 128 - DH, NTILE + t, t)
            t_hi = pl.multiple_of(t * 128, 128)
            t_lo = pl.multiple_of(jnp.minimum(t + 1, NTILE - 1) * 128, 128)
            r = lax.broadcasted_iota(jnp.int32, (128, TQ), 0)
            head_bits = jnp.where(((r - lo) & 127) < DH, -1, zero_ref[0, 0])
            upper = r >= lo
            lag = PACE_FIRST if first else PACE
            if vpu:
                kr = vpu_keys(jnp.minimum(h1 + 1, H - 1))
        if h2 is not None:
            off = 4 * par
            w0 = pl.multiple_of(h2 * DH - off, 8)
            rv = lax.broadcasted_iota(jnp.int32, (VROWS, S), 0)
            vt = jnp.where((rv >= off) & (rv < off + DH), vt_ref[pl.ds(w0, VROWS), :], 1.0)
            ro = lax.broadcasted_iota(jnp.int32, (VROWS, TQ), 0)
            ovalid = (ro >= off) & (ro < off + DH)
            lrow = DH if par == 0 else 0
        for ui, u in enumerate(range(NQ) if blocks is None else blocks):
            cols = cols_of(u)
            if h1 is not None:
                qw = jnp.where(upper, qt_ref[u, pl.ds(t_hi, 128), :], qt_ref[u, pl.ds(t_lo, 128), :])
                qw = pltpu.bitcast(pltpu.bitcast(qw, jnp.int32) & head_bits, F32)
            if h2 is not None:
                m2 = mx_ref[par, u]
            m = None
            acc = None
            for c in range(NC):
                ks = slice(c * TK, (c + 1) * TK)
                if h1 is not None:
                    kb = kf_ref[h1, c] if first else kb_refs[par][c]
                    if len(pace) >= lag:
                        zs = pltpu.bitcast(pace[-lag][0:8, :], jnp.int32) & zv_ref[...]
                        kb0 = pltpu.bitcast(pltpu.bitcast(kb[0], jnp.int32) | zs, F32)
                        kb = jnp.concatenate([kb0[None], kb[1:]], axis=0)
                    sv = jnp.sum(kb * (qf_ref[h1, u] if first else qb_refs[par][u]), axis=0)
                if h2 is not None:
                    s = s_ref[par, u, ks, :]
                    p = jnp.exp2(s.reshape(TK // 8, 8, TQ) - m2[None]).reshape(TK, TQ)
                    d = _dot(vt[:, ks], p)
                    acc = d if acc is None else acc + d
                if h1 is not None:
                    s = _dot(k_ref[ktile, c * TK + VR:(c + 1) * TK, :], qw)
                    pace.append(s)
                    s = jnp.concatenate([sv, s], axis=0)
                    s_ref[par, u, ks, :] = s
                    mc = jnp.max(s.reshape(TK // 8, 8, TQ), axis=0)
                    m = mc if m is None else jnp.maximum(m, mc)
                if extra is not None:
                    extra(ui, c)
            if h1 is not None:
                m = jnp.max(m, axis=0, keepdims=True)
                mx_ref[par, u] = jnp.broadcast_to(m, (8, TQ))
                if vpu:
                    build_qb(jnp.minimum(h1 + 2, H - 2 + par), par, u)
                    if 2 * u < DH:
                        zm = pltpu.bitcast(jnp.broadcast_to(m, (8, TQ)), jnp.int32) & zv_ref[...]
                        krz = pltpu.bitcast(pltpu.bitcast(kr, jnp.int32) | jnp.tile(zm, (NC, 1)), F32)
                        build_kb(krz, 1 - par, (2 * u, 2 * u + 1))
            if h2 is not None:
                o = acc / acc[lrow:lrow + 1, :]
                if outs is None:
                    pltpu.store(ot_ref.at[pl.ds(w0, VROWS), cols], o, mask=ovalid)
                else:
                    outs.append(o)

    def last_heads(j):
        base = pl.multiple_of(j * 2 * RB, 2 * RB)
        quarter = [pl.ds(base + i * 128, 128) for i in range(4)]
        o = [ot_ref[0:512, r].T.astype(BF16) for r in quarter]

        outs = ([], [])

        def piece(i, n, k):
            x_ref[quarter[i], n * 128:(n + 1) * 128] += _dot(
                o[i][:, k * 256:(k + 1) * 256], wbo_ref[k * 256:(k + 1) * 256, n * 128:(n + 1) * 128])

        def finish(i):
            r = quarter[i]
            oa, ob = outs[0][i], outs[1][i]
            sub = lax.broadcasted_iota(jnp.int32, (8, TQ), 0)
            last = jnp.concatenate([ot_ref[512:D - 2 * DH, r], oa[0:16, :],
                                    jnp.where(sub < 4, oa[16:24, :], ob[0:8, :]), ob[8:24, :]], axis=0)
            xb = x_ref[r, :] + _dot(last.T.astype(BF16), wbo_ref[512:D, :])
            x_ref[r, :] = xb
            xin_ref[r, :] = xb.astype(BF16)
            if i % 2 == 1:
                out_copy(2 * j + i // 2).start()

        def pieces(b):
            return [(piece, (i, n, k)) for k in range(2) for i in (2 * b, 2 * b + 1) for n in range(NTILE)]
        jobs = pieces(0) + pieces(1)[:4] + [(finish, (0,)), (finish, (1,))] + pieces(1)[4:]
        jobs += [(finish, (2,)), (finish, (3,))]
        n_in = len(jobs) - TAIL_LEFT
        slots = [TAIL_FIRST + (t * (8 * NC - TAIL_FIRST)) // n_in for t in range(n_in)]

        def extra(first):
            def f(ui, c):
                step = first + ui * NC + c
                while step in slots:
                    fn, args = jobs[slots.index(step)]
                    slots[slots.index(step)] = -1
                    fn(*args)
            return f
        for b in range(2):
            blocks = [4 * j + 2 * b, 4 * j + 2 * b + 1]
            attn(None, H - 2, 0, extra(4 * b * NC), blocks=blocks, outs=outs[0])
            attn(None, H - 1, 1, extra((4 * b + 2) * NC), blocks=blocks, outs=outs[1])
        for fn, args in jobs[n_in:]:
            fn(*args)

    cp_wak.start()
    x_copy(0).start()
    cp_waq.start()
    x_copy(1).start()
    x_copy(2).start()
    g_ref[...] = jnp.zeros(g_ref.shape, F32)
    zp_ref[...] = jnp.zeros(zp_ref.shape, F32)
    zv_ref[...] = jnp.zeros(zv_ref.shape, jnp.int32)
    zero_ref[0, 0] = 0
    cp_wak.wait()
    for b in range(3, NB):
        x_copy(b).start()
    cp_wav.start()
    cp_wao.start()
    cp_wb.start()
    cp_wbo.start()
    wat_ref[0:D, :] = wa_ref[:, D:2 * D].astype(F32).T.astype(BF16)
    x_copy(0).wait()
    x0 = xin_ref[rows_of(0), :].astype(F32)
    x_ref[rows_of(0), :] = x0
    xn_ref[...] = _layernorm(x0)
    cp_waq.wait()
    wat_ref[D:2 * D, :] = wa_ref[:, 0:D].astype(F32).T.astype(BF16)

    def two_layers(it, c):
        first = it == 0

        def load_x(b):
            rows = rows_of(b)
            xb = jnp.where(first, xin_ref[rows, :].astype(F32), x_ref[rows, :])
            x_ref[rows, :] = xb
            return _layernorm(xb)

        def a1_body(j, c):
            @pl.when(first)
            def _():
                x_copy(2 * j + 1).wait()

                @pl.when(j < NIT - 1)
                def _():
                    x_copy(2 * j + 2).wait()
            a1_pair(j, load_x)
            return c
        lax.fori_loop(0, NIT, a1_body, 0)

        @pl.when(first)
        def _():
            cp_wav.wait()
            cp_wao.wait()
            cp_wb.wait()
            cp_wbo.wait()

        @pl.when(jnp.logical_not(first))
        def _():
            for b in range(NB):
                out_copy(b).wait()

        wbt_ref[0:D, :] = wb_ref[:, 0:D].astype(F32).T.astype(BF16)
        wbt_ref[D:2 * D, :] = wb_ref[:, 2 * D:3 * D].astype(F32).T.astype(BF16)
        xn_ref[...] = _layernorm(a3_x(0, a2()))

        def a3_b1(b, c):
            y = a3_y(b + 1)
            b1_k(b, xn_ref[...])
            xn_next = _layernorm(a3_x(b + 1, y))
            b1_qv(b, xn_ref[...])
            xn_ref[...] = xn_next
            return c
        lax.fori_loop(0, NB - 1, a3_b1, 0)
        b1_k(NB - 1, xn_ref[...])
        b1_qv(NB - 1, xn_ref[...])

        def first_scores(h, c):
            attn(h, None, h, pace=[], first=True)
            return c
        lax.fori_loop(0, 2, first_scores, 0)

        def body(i, c):
            pace = []
            attn(2 * i + 2, 2 * i, 0, vpu=True, pace=pace)
            attn(2 * i + 3, 2 * i + 1, 1, vpu=True, pace=pace)
            return c
        lax.fori_loop(0, H // 2 - 1, body, 0)

        def tail(j, c):
            last_heads(j)
            return c
        lax.fori_loop(0, NIT, tail, 0)

        @pl.when(first)
        def _():
            xn_ref[...] = _layernorm(x_ref[rows_of(0), :])
        return c
    lax.fori_loop(0, 2, two_layers, 0)
    for b in range(NB):
        out_copy(b).wait()


@jax.jit
def pallas_interleave_layers__linear_attn_block__mha_block__prompt_kernel(
    A_x: jax.Array,
    A_wqkv: jax.Array,
    A_wo: jax.Array,
    B_x: jax.Array,
    B_wqkv: jax.Array,
    B_wo: jax.Array,
):
    del B_x
    x = A_x.reshape(S, D)
    any_spec = pl.BlockSpec(memory_space=pl.ANY)
    out = pl.pallas_call(
        _kernel,
        out_shape=jax.ShapeDtypeStruct((S, D), BF16),
        in_specs=[any_spec] * 5,
        out_specs=any_spec,
        scratch_shapes=[
            pltpu.VMEM((S, D), BF16),
            pltpu.VMEM((D, 3 * D), BF16),
            pltpu.VMEM((D, D), BF16),
            pltpu.VMEM((D, 3 * D), BF16),
            pltpu.VMEM((D, D), BF16),
            pltpu.SemaphoreType.DMA((NB + 6,)),
            pltpu.VMEM((S, D), F32),
            pltpu.VMEM((RB, D), BF16),
            pltpu.VMEM((2 * D, D), BF16),
            pltpu.VMEM((2 * D, D), BF16),
            pltpu.VMEM((D, S), F32),
            pltpu.VMEM((D, D), F32),
            pltpu.VMEM((D, 128), F32),
            pltpu.VMEM((D, D), BF16),
            pltpu.VMEM((H, D), F32),
            pltpu.VMEM((NQ, D, TQ), F32),
            pltpu.VMEM((2 * NTILE - 1, S, 128), F32),
            pltpu.VMEM((D, S), F32),
            pltpu.VMEM((D, S), F32),
            pltpu.VMEM((2, NQ, S, TQ), F32),
            pltpu.VMEM((2, NQ, 8, TQ), F32),
            pltpu.VMEM((NQ, DH, 8, TQ), F32),
            pltpu.VMEM((NQ, DH, 8, TQ), F32),
            pltpu.VMEM((NC, DH, VR, TQ), F32),
            pltpu.VMEM((NC, DH, VR, TQ), F32),
            pltpu.VMEM((2, NC, DH, VR, TQ), F32),
            pltpu.VMEM((2, NQ, DH, 8, TQ), F32),
            pltpu.VMEM((8, TQ), jnp.int32),
            pltpu.SMEM((1, 1), jnp.int32),
        ],
        compiler_params=pltpu.CompilerParams(vmem_limit_bytes=110 * 1024 * 1024),
    )(x, A_wqkv, A_wo, B_wqkv, B_wo)
    return out.reshape(1, S, D)
```

```python
import jax
import jax.numpy as jnp
from jax import lax
import jax.experimental.pallas as pl
import jax.experimental.pallas.tpu as pltpu

S = 2048
D = 640
H = 32
DH = 20
NTILE = D // 128
RB = 256
NB = S // RB
NIT = NB // 2
TQ = 128
TK = 128
NQ = S // TQ
NC = S // TK
VR = 8
PACE = 5
PACE_FIRST = 5
TAIL_FIRST = 6
TAIL_LEFT = 10
VROWS = 24
KV_ROWS = ((0, 144), (112, 272), (240, 400), (368, 528), (496, 640))

LOG2E = 1.4426950408889634
QSCALE = (DH ** -0.5) * LOG2E

F32 = jnp.float32
BF16 = jnp.bfloat16
_NT = (((1,), (1,)), ((), ()))


def _dot(a, b):
    return jnp.dot(a, b, preferred_element_type=F32)


def _dot_nt(a, b):
    return lax.dot_general(a, b, _NT, preferred_element_type=F32)


def _layernorm(xb):
    m = jnp.mean(xb, axis=-1, keepdims=True)
    xc = xb - m
    v = jnp.mean(xc * xc, axis=-1, keepdims=True)
    return (xc * lax.rsqrt(v + 1e-5)).astype(BF16)


def _phi(t):
    return jnp.where(t > 0, t + 1.0, jnp.exp(t)) + 1e-6


def _kernel(x_hbm, wa_hbm, wao_hbm, wb_hbm, wbo_hbm, out_hbm,
            xin_ref, wa_ref, wao_ref, wb_ref, wbo_ref, sems,
            x_ref, xn_ref, wat_ref, wbt_ref, pq_ref, g_ref, zp_ref, m_ref, zh_ref,
            qt_ref, k_ref, vt_ref, ot_ref, s_ref, mx_ref,
            qb0_ref, qb1_ref, kb0_ref, kb1_ref, kf_ref, qf_ref, zv_ref):
    qb_refs = (qb0_ref, qb1_ref)
    kb_refs = (kb0_ref, kb1_ref)

    def rows_of(b):
        if isinstance(b, int):
            return slice(b * RB, (b + 1) * RB)
        return pl.ds(pl.multiple_of(b * RB, RB), RB)

    def x_copy(b):
        return pltpu.make_async_copy(x_hbm.at[rows_of(b), :], xin_ref.at[rows_of(b), :], sems.at[b])

    def out_copy(b):
        return pltpu.make_async_copy(xin_ref.at[rows_of(b), :], out_hbm.at[rows_of(b), :], sems.at[b])

    cp_wak = pltpu.make_async_copy(wa_hbm.at[:, pl.ds(D, D)], wa_ref.at[:, pl.ds(D, D)], sems.at[NB])
    cp_waq = pltpu.make_async_copy(wa_hbm.at[:, pl.ds(0, D)], wa_ref.at[:, pl.ds(0, D)], sems.at[NB + 1])
    cp_wav = pltpu.make_async_copy(wa_hbm.at[:, pl.ds(2 * D, D)], wa_ref.at[:, pl.ds(2 * D, D)],
                                   sems.at[NB + 2])
    cp_wao = pltpu.make_async_copy(wao_hbm, wao_ref, sems.at[NB + 3])
    cp_wb = pltpu.make_async_copy(wb_hbm, wb_ref, sems.at[NB + 4])
    cp_wbo = pltpu.make_async_copy(wbo_hbm, wbo_ref, sems.at[NB + 5])

    def a1_stage(b, xn):
        pkt = _phi(_dot_nt(wat_ref[0:D, :], xn))
        pq_ref[:, rows_of(b)] = _phi(_dot_nt(wat_ref[D:2 * D, :], xn))
        zp = pkt[:, 0:128]
        for t in range(1, RB // 128):
            zp = zp + pkt[:, t * 128:(t + 1) * 128]
        return zp, _dot(pkt.astype(BF16), xn)

    def a1_pair(j, ln_of):
        xn_b = ln_of(2 * j + 1)
        zp0, g0 = a1_stage(2 * j, xn_ref[...])
        xn_ref[...] = ln_of(jnp.minimum(2 * j + 2, NB - 1))
        zp1, g1 = a1_stage(2 * j + 1, xn_b)
        zp_ref[...] += zp0 + zp1
        g_ref[...] += g0 + g1

    def a2():
        z = jnp.sum(zp_ref[...].T, axis=0, keepdims=True)
        hj = lax.broadcasted_iota(jnp.int32, (H, D), 0) * DH
        cd = lax.broadcasted_iota(jnp.int32, (H, D), 1)
        zh_ref[...] = jnp.where((cd >= hj) & (cd < hj + DH), z, 0.0)
        kvm = []
        for t, (lo, hi) in enumerate(KV_ROWS):
            n = hi - lo
            kv = _dot(g_ref[lo:hi, :].astype(BF16), wa_ref[:, 2 * D + t * 128:2 * D + (t + 1) * 128])
            rd = lax.broadcasted_iota(jnp.int32, (n, 128), 0) + lo
            ce = lax.broadcasted_iota(jnp.int32, (n, 128), 1) + t * 128
            h0 = ((rd * 3277) >> 16) * DH
            kvm.append(jnp.where((ce >= h0) & (ce < h0 + DH), kv, 0.0).astype(BF16))
        y0 = a3_y(0)
        mt = [_dot(kvm[t], wao_ref[t * 128:(t + 1) * 128, :]) for t in range(NTILE)]
        for t, (lo, hi) in enumerate(KV_ROWS):
            a = KV_ROWS[t - 1][1] if t > 0 else lo
            b = KV_ROWS[t + 1][0] if t + 1 < NTILE else hi
            m_ref[a:b, :] = mt[t][a - lo:b - lo, :].astype(BF16)
            if b < hi:
                m_ref[b:hi, :] = (mt[t][b - lo:, :] + mt[t + 1][0:hi - b, :]).astype(BF16)
        g_ref[...] = jnp.zeros(g_ref.shape, F32)
        zp_ref[...] = jnp.zeros(zp_ref.shape, F32)
        return y0

    def a3_y(b):
        rows = rows_of(b)
        r = 1.0 / (_dot(zh_ref[...], pq_ref[:, rows]) + 1e-6)
        sub = lax.broadcasted_iota(jnp.int32, (8, RB), 0)
        pieces = []
        for j in range(H // 2):
            ra = jnp.broadcast_to(r[2 * j:2 * j + 1, :], (8, RB))
            rb = jnp.broadcast_to(r[2 * j + 1:2 * j + 2, :], (8, RB))
            pieces += [ra, ra, jnp.where(sub < 4, ra, rb), rb, rb]
        return (pq_ref[:, rows] * jnp.concatenate(pieces, axis=0)).T.astype(BF16)

    def a3_x(b, y):
        xb = x_ref[rows_of(b), :] + _dot(y, m_ref[...])
        x_ref[rows_of(b), :] = xb
        return xb

    def b1_k(b, xn):
        rows = rows_of(b)
        k = _dot(xn, wb_ref[:, D:2 * D])
        lane = lax.broadcasted_iota(jnp.int32, (RB, 128), 1)
        for t in range(NTILE):
            k_ref[t, rows, :] = k[:, t * 128:(t + 1) * 128]
        for t in range(NTILE - 1):
            k_ref[NTILE + t, rows, :] = jnp.where(
                lane >= 64, k[:, t * 128:(t + 1) * 128],
                k[:, (t + 1) * 128:(t + 2) * 128])

        for i in range(RB // TK):
            c = b * (RB // TK) + i
            kr = k[i * TK:i * TK + VR, 0:128]
            for d in range(2 * DH):
                kf_ref[d // DH, c, d % DH] = jnp.broadcast_to(kr[:, d:d + 1], (VR, TQ))
            for dd in range(DH):
                kb_refs[0][c, dd] = jnp.broadcast_to(kr[:, 2 * DH + dd:2 * DH + dd + 1], (VR, TQ))

    def b1_qv(b, xn):
        rows = rows_of(b)
        qvt = _dot_nt(wbt_ref[...], xn)
        for i in range(RB // TQ):
            qs = qvt[0:D, i * TQ:(i + 1) * TQ] * QSCALE
            qt_ref[b * (RB // TQ) + i] = qs
            for d in range(2 * DH):
                qf_ref[d // DH, b * (RB // TQ) + i, d % DH] = jnp.broadcast_to(qs[d:d + 1, :], (8, TQ))
            for par in range(2):
                for dd in range(DH):
                    r = (2 + par) * DH + dd
                    qb_refs[par][b * (RB // TQ) + i, dd] = jnp.broadcast_to(qs[r:r + 1, :], (8, TQ))
        vt_ref[:, rows] = qvt[D:2 * D, :]

    def cols_of(u):
        if isinstance(u, int):
            return slice(u * TQ, (u + 1) * TQ)
        return pl.ds(pl.multiple_of(u * TQ, TQ), TQ)

    def build_qb(h, par, u):
        win = qt_ref[u, pl.ds(pl.multiple_of(h * DH - 4 * par, 8), VROWS), :]
        for dd in range(DH):
            r = 4 * par + dd
            qb_refs[par][u, dd] = jnp.broadcast_to(win[r:r + 1, :], (8, TQ))

    def vpu_keys(h):
        d0 = h * DH
        lo = d0 & 127
        ktile = jnp.where(lo > 128 - DH, NTILE + (d0 >> 7), d0 >> 7)
        rows = jnp.concatenate([k_ref[ktile, c * TK:c * TK + VR, :] for c in range(NC)], axis=0)
        return pltpu.roll(rows, (128 - lo) & 127, axis=1)

    def build_kb(kr, par, ds, zero):
        for dd in ds:
            kbd = jnp.broadcast_to(kr[:, dd:dd + 1], (NC * VR, TQ))
            kb_refs[par][:, dd + zero] = kbd.reshape(NC, VR, TQ)

    def attn(h1, h2, par, extra=None, blocks=None, vpu=False, pace=None, outs=None, first=False):
        if h1 is not None:
            d0 = h1 * DH
            t = d0 >> 7
            lo = d0 & 127
            ktile = jnp.where(lo > 128 - DH, NTILE + t, t)
            t_hi = pl.multiple_of(t * 128, 128)
            t_lo = pl.multiple_of(jnp.minimum(t + 1, NTILE - 1) * 128, 128)
            r = lax.broadcasted_iota(jnp.int32, (128, TQ), 0)
            zero = h1 >> 16
            head_bits = jnp.where(((r - lo) & 127) < DH, -1, zero)
            upper = r >= lo
            lag = PACE_FIRST if first else PACE
            if vpu:
                kr = vpu_keys(jnp.minimum(h1 + 1, H - 1))
        if h2 is not None:
            off = 4 * par
            w0 = pl.multiple_of(h2 * DH - off, 8)
            rv = lax.broadcasted_iota(jnp.int32, (VROWS, S), 0)
            vt = jnp.where((rv >= off) & (rv < off + DH), vt_ref[pl.ds(w0, VROWS), :], 1.0)
            ro = lax.broadcasted_iota(jnp.int32, (VROWS, TQ), 0)
            ovalid = (ro >= off) & (ro < off + DH)
            lrow = DH if par == 0 else 0
        for ui, u in enumerate(range(NQ) if blocks is None else blocks):
            cols = cols_of(u)
            if h1 is not None:
                qw = jnp.where(upper, qt_ref[u, pl.ds(t_hi, 128), :], qt_ref[u, pl.ds(t_lo, 128), :])
                qw = pltpu.bitcast(pltpu.bitcast(qw, jnp.int32) & head_bits, F32)
            if h2 is not None:
                m2 = mx_ref[par, u]
            m = None
            acc = None
            for c in range(NC):
                ks = slice(c * TK, (c + 1) * TK)
                if h1 is not None:
                    kb = kf_ref[h1, c] if first else kb_refs[par][c]
                    if len(pace) >= lag:
                        zs = pltpu.bitcast(pace[-lag][0:8, :], jnp.int32) & zv_ref[...]
                        kb0 = pltpu.bitcast(pltpu.bitcast(kb[0], jnp.int32) | zs, F32)
                        kb = jnp.concatenate([kb0[None], kb[1:]], axis=0)
                    sv = jnp.sum(kb * (qf_ref[h1, u] if first else qb_refs[par][u]), axis=0)
                if h2 is not None:
                    s = s_ref[par, u, ks, :]
                    p = jnp.exp2(s.reshape(TK // 8, 8, TQ) - m2[None]).reshape(TK, TQ)
                    d = _dot(vt[:, ks], p)
                    acc = d if acc is None else acc + d
                if h1 is not None:
                    s = _dot(k_ref[ktile, c * TK + VR:(c + 1) * TK, :], qw)
                    pace.append(s)
                    s = jnp.concatenate([sv, s], axis=0)
                    s_ref[par, u, ks, :] = s
                    mc = jnp.max(s.reshape(TK // 8, 8, TQ), axis=0)
                    m = mc if m is None else jnp.maximum(m, mc)
                if extra is not None:
                    extra(ui, c)
            if h1 is not None:
                m = jnp.max(m, axis=0, keepdims=True)
                mx_ref[par, u] = jnp.broadcast_to(m, (8, TQ))
                if vpu:
                    build_qb(jnp.minimum(h1 + 2, H - 2 + par), par, u)
                    if 2 * u < DH:
                        zm = pltpu.bitcast(jnp.broadcast_to(m, (8, TQ)), jnp.int32) & zv_ref[...]
                        krz = pltpu.bitcast(pltpu.bitcast(kr, jnp.int32) | jnp.tile(zm, (NC, 1)), F32)
                        build_kb(krz, 1 - par, (2 * u, 2 * u + 1), zero)
            if h2 is not None:
                o = acc / acc[lrow:lrow + 1, :]
                if outs is None:
                    pltpu.store(ot_ref.at[pl.ds(w0, VROWS), cols], o, mask=ovalid)
                else:
                    outs.append(o)

    def last_heads(j):
        base = pl.multiple_of(j * 2 * RB, 2 * RB)
        quarter = [pl.ds(base + i * 128, 128) for i in range(4)]
        o = [ot_ref[0:512, r].T.astype(BF16) for r in quarter]

        outs = ([], [])

        def piece(i, n, k):
            x_ref[quarter[i], n * 128:(n + 1) * 128] += _dot(
                o[i][:, k * 256:(k + 1) * 256], wbo_ref[k * 256:(k + 1) * 256, n * 128:(n + 1) * 128])

        def finish(i):
            r = quarter[i]
            oa, ob = outs[0][i], outs[1][i]
            sub = lax.broadcasted_iota(jnp.int32, (8, TQ), 0)
            last = jnp.concatenate([ot_ref[512:D - 2 * DH, r], oa[0:16, :],
                                    jnp.where(sub < 4, oa[16:24, :], ob[0:8, :]), ob[8:24, :]], axis=0)
            xb = x_ref[r, :] + _dot(last.T.astype(BF16), wbo_ref[512:D, :])
            x_ref[r, :] = xb
            xin_ref[r, :] = xb.astype(BF16)
            if i % 2 == 1:
                out_copy(2 * j + i // 2).start()

        def pieces(b):
            return [(piece, (i, n, k)) for k in range(2) for i in (2 * b, 2 * b + 1) for n in range(NTILE)]
        jobs = pieces(0) + pieces(1)[:4] + [(finish, (0,)), (finish, (1,))] + pieces(1)[4:]
        jobs += [(finish, (2,)), (finish, (3,))]
        n_in = len(jobs) - TAIL_LEFT
        slots = [TAIL_FIRST + (t * (8 * NC - TAIL_FIRST)) // n_in for t in range(n_in)]

        def extra(first):
            def f(ui, c):
                step = first + ui * NC + c
                while step in slots:
                    fn, args = jobs[slots.index(step)]
                    slots[slots.index(step)] = -1
                    fn(*args)
            return f
        for b in range(2):
            blocks = [4 * j + 2 * b, 4 * j + 2 * b + 1]
            attn(None, H - 2, 0, extra(4 * b * NC), blocks=blocks, outs=outs[0])
            attn(None, H - 1, 1, extra((4 * b + 2) * NC), blocks=blocks, outs=outs[1])
        for fn, args in jobs[n_in:]:
            fn(*args)

    cp_wak.start()
    x_copy(0).start()
    cp_waq.start()
    x_copy(1).start()
    x_copy(2).start()
    g_ref[...] = jnp.zeros(g_ref.shape, F32)
    zp_ref[...] = jnp.zeros(zp_ref.shape, F32)
    zv_ref[...] = jnp.zeros(zv_ref.shape, jnp.int32)
    cp_wak.wait()
    for b in range(3, NB):
        x_copy(b).start()
    cp_wav.start()
    cp_wao.start()
    cp_wb.start()
    cp_wbo.start()
    wat_ref[0:D, :] = wa_ref[:, D:2 * D].astype(F32).T.astype(BF16)
    x_copy(0).wait()
    x0 = xin_ref[rows_of(0), :].astype(F32)
    x_ref[rows_of(0), :] = x0
    xn_ref[...] = _layernorm(x0)
    cp_waq.wait()
    wat_ref[D:2 * D, :] = wa_ref[:, 0:D].astype(F32).T.astype(BF16)

    def two_layers(it, c):
        first = it == 0

        def load_x(b):
            rows = rows_of(b)
            xb = jnp.where(first, xin_ref[rows, :].astype(F32), x_ref[rows, :])
            x_ref[rows, :] = xb
            return _layernorm(xb)

        def a1_body(j, c):
            @pl.when(first)
            def _():
                x_copy(2 * j + 1).wait()

                @pl.when(j < NIT - 1)
                def _():
                    x_copy(jnp.minimum(2 * j + 2, NB - 1)).wait()
            a1_pair(j, load_x)
            return c
        lax.fori_loop(0, NIT, a1_body, 0)

        @pl.when(first)
        def _():
            cp_wav.wait()
            cp_wao.wait()
            cp_wb.wait()
            cp_wbo.wait()

        @pl.when(jnp.logical_not(first))
        def _():
            for b in range(NB):
                out_copy(b).wait()

        wbt_ref[0:D, :] = wb_ref[:, 0:D].astype(F32).T.astype(BF16)
        wbt_ref[D:2 * D, :] = wb_ref[:, 2 * D:3 * D].astype(F32).T.astype(BF16)
        xn_ref[...] = _layernorm(a3_x(0, a2()))

        def a3_b1(b, c):
            y = a3_y(b + 1)
            b1_k(b, xn_ref[...])
            xn_next = _layernorm(a3_x(b + 1, y))
            b1_qv(b, xn_ref[...])
            xn_ref[...] = xn_next
            return c
        lax.fori_loop(0, NB - 1, a3_b1, 0)
        b1_k(NB - 1, xn_ref[...])
        b1_qv(NB - 1, xn_ref[...])

        def first_scores(h, c):
            attn(h, None, h, pace=[], first=True)
            return c
        lax.fori_loop(0, 2, first_scores, 0)

        def body(i, c):
            pace = []
            attn(2 * i + 2, 2 * i, 0, vpu=True, pace=pace)
            attn(2 * i + 3, 2 * i + 1, 1, vpu=True, pace=pace)
            return c
        lax.fori_loop(0, H // 2 - 1, body, 0)

        def tail(j, c):
            last_heads(j)
            return c
        lax.fori_loop(0, NIT, tail, 0)

        @pl.when(first)
        def _():
            xn_ref[...] = _layernorm(x_ref[rows_of(0), :])
        return c
    lax.fori_loop(0, 2, two_layers, 0)
    for b in range(NB):
        out_copy(b).wait()


@jax.jit
def pallas_interleave_layers__linear_attn_block__mha_block__prompt_kernel(
    A_x: jax.Array,
    A_wqkv: jax.Array,
    A_wo: jax.Array,
    B_x: jax.Array,
    B_wqkv: jax.Array,
    B_wo: jax.Array,
):
    del B_x
    x = A_x.reshape(S, D)
    any_spec = pl.BlockSpec(memory_space=pl.ANY)
    out = pl.pallas_call(
        _kernel,
        out_shape=jax.ShapeDtypeStruct((S, D), BF16),
        in_specs=[any_spec] * 5,
        out_specs=any_spec,
        scratch_shapes=[
            pltpu.VMEM((S, D), BF16),
            pltpu.VMEM((D, 3 * D), BF16),
            pltpu.VMEM((D, D), BF16),
            pltpu.VMEM((D, 3 * D), BF16),
            pltpu.VMEM((D, D), BF16),
            pltpu.SemaphoreType.DMA((NB + 6,)),
            pltpu.VMEM((S, D), F32),
            pltpu.VMEM((RB, D), BF16),
            pltpu.VMEM((2 * D, D), BF16),
            pltpu.VMEM((2 * D, D), BF16),
            pltpu.VMEM((D, S), F32),
            pltpu.VMEM((D, D), F32),
            pltpu.VMEM((D, 128), F32),
            pltpu.VMEM((D, D), BF16),
            pltpu.VMEM((H, D), F32),
            pltpu.VMEM((NQ, D, TQ), F32),
            pltpu.VMEM((2 * NTILE - 1, S, 128), F32),
            pltpu.VMEM((D, S), F32),
            pltpu.VMEM((D, S), F32),
            pltpu.VMEM((2, NQ, S, TQ), F32),
            pltpu.VMEM((2, NQ, 8, TQ), F32),
            pltpu.VMEM((NQ, DH, 8, TQ), F32),
            pltpu.VMEM((NQ, DH, 8, TQ), F32),
            pltpu.VMEM((NC, DH, VR, TQ), F32),
            pltpu.VMEM((NC, DH, VR, TQ), F32),
            pltpu.VMEM((2, NC, DH, VR, TQ), F32),
            pltpu.VMEM((2, NQ, DH, 8, TQ), F32),
            pltpu.VMEM((8, TQ), jnp.int32),
        ],
        compiler_params=pltpu.CompilerParams(vmem_limit_bytes=110 * 1024 * 1024),
    )(x, A_wqkv, A_wo, B_wqkv, B_wo)
    return out.reshape(1, S, D)
```
